```python
import jax
import jax.numpy as jnp

def _softmax(x, axis=-1):
    return jax.nn.softmax(x, axis=axis)

def _gelu(x):
    return jax.nn.gelu(x, approximate=True)

def _silu(x):
    return jax.nn.silu(x)

def _sigmoid(x):
    return jax.nn.sigmoid(x)

def _layernorm(x, axis=-1, eps=1e-05):
    m = jnp.mean(x, axis=axis, keepdims=True)
    v = jnp.var(x, axis=axis, keepdims=True)
    return (x - m) / jnp.sqrt(v + eps)

def _scatter_add(tgt, idx, src, axis=0):
    return tgt.at[idx].add(src)

def _segment_sum(src, seg, n):
    return jax.ops.segment_sum(src, seg, n)

class _Rng:

    def __init__(self, key):
        self._k = key

    def _next(self):
        self._k, sub = jax.random.split(self._k)
        return sub

    def normal(self, shape):
        return jax.random.normal(self._next(), shape, dtype=jnp.bfloat16)

    def randint(self, lo, hi, shape):
        return jax.random.randint(self._next(), shape, lo, hi, dtype=jnp.int32)

    def uniform(self, shape, lo=0.0, hi=1.0):
        return jax.random.uniform(self._next(), shape, jnp.bfloat16, lo, hi)

    def permutation(self, n):
        return jax.random.permutation(self._next(), n)
kernel_name = 'standalone__autoregressive_conv_wavernn__speech'

def setup_inputs():
    _rng = _Rng(jax.random.key(int.from_bytes(__import__("os").urandom(4), "little")))
    _w = lambda a: (lambda t: t.astype(jnp.bfloat16) if jnp.issubdtype(t.dtype, jnp.floating) else t)(jnp.asarray(a))
    B, T, D, K = (2, 16000, 256, 31)
    return {'x': _w((lambda *s: _rng.normal(s) * 0.05)(B, T, D)), 'w': _w((lambda *s: _rng.normal(s) * 0.05)(K, D, 2 * D))}

def reference(x, w):
    B, T, D = x.shape
    K = w.shape[0]
    dil = 2
    pad = (K - 1) * dil
    xp = jnp.pad(x, ((0, 0), (pad, 0), (0, 0)))
    h = jnp.einsum('btd,de->bte', xp[:, 0:T, :], w[0])
    for i in range(1, K):
        h = h + jnp.einsum('btd,de->bte', xp[:, i * dil:i * dil + T, :], w[i])
    f, g = (h[..., :D].copy(), h[..., D:].copy())
    return jnp.tanh(f) * _sigmoid(g)
```

```python
import jax
import jax.numpy as jnp
import jax.experimental.pallas as pl
import jax.experimental.pallas.tpu as pltpu

_TT = 800


def _kern(xprev_ref, x_ref, w_ref, o_ref, xs_ref):
    tt = _TT
    t = pl.program_id(1)
    K = w_ref.shape[0]
    D = x_ref.shape[-1]
    halo = xprev_ref[tt - 64:, :]
    halo = jnp.where(t > 0, halo, jnp.zeros_like(halo))
    xs_ref[0:64, :] = halo
    xs_ref[64:, :] = x_ref[...]
    acc = jnp.zeros((tt, 2 * D), jnp.float32)
    for i in range(K):
        off = 4 + 2 * i
        acc = acc + jnp.dot(xs_ref[off:off + tt, :], w_ref[i],
                            preferred_element_type=jnp.float32)
    f = acc[:, :D]
    g = acc[:, D:]
    o_ref[...] = (jnp.tanh(f) * jax.nn.sigmoid(g)).astype(o_ref.dtype)


@jax.jit
def pallas_standalone__autoregressive_conv_wavernn__speech_kernel(
    x: jax.Array,
    w: jax.Array,
):
    B, T, D = x.shape
    K = w.shape[0]
    tt = _TT
    return pl.pallas_call(
        _kern,
        grid=(B, T // tt),
        in_specs=[
            pl.BlockSpec((None, tt, D), lambda b, t: (b, jnp.maximum(t - 1, 0), 0)),
            pl.BlockSpec((None, tt, D), lambda b, t: (b, t, 0)),
            pl.BlockSpec((K, D, 2 * D), lambda b, t: (0, 0, 0)),
        ],
        out_specs=pl.BlockSpec((None, tt, D), lambda b, t: (b, t, 0)),
        out_shape=jax.ShapeDtypeStruct((B, T, D), x.dtype),
        scratch_shapes=[pltpu.VMEM((tt + 64, D), x.dtype)],
        compiler_params=pltpu.CompilerParams(
            dimension_semantics=("parallel", "arbitrary"),
            vmem_limit_bytes=100 * 1024 * 1024),
    )(x, x, w)
```

```python
import math
import numpy as np
import jax
import jax.numpy as jnp
from jax.experimental import pallas as pl
from jax.experimental.pallas import tpu as pltpu

def vneg(a):
    return None if a is None else (a[0], -a[1])


def vadd(a, b):
    if a is None:
        return b
    if b is None:
        return a
    if a[1] > 0 and b[1] > 0:
        return (a[0] + b[0], 1)
    if a[1] > 0 and b[1] < 0:
        return (a[0] - b[0], 1)
    if a[1] < 0 and b[1] > 0:
        return (b[0] - a[0], 1)
    return (a[0] + b[0], -1)


def vsub(a, b):
    return vadd(a, vneg(b))


def vmulc(a, c):
    if a is None or c == 0.0:
        return None
    if c == 1.0:
        return a
    if c == -1.0:
        return vneg(a)
    return (a[0] * float(np.float32(c * a[1])), 1)


def vmat(a):
    return a[0] if a[1] > 0 else -a[0]


def cadd(a, b):
    return (vadd(a[0], b[0]), vadd(a[1], b[1]))


def csub(a, b):
    return (vsub(a[0], b[0]), vsub(a[1], b[1]))


def conj(a):
    return (a[0], vneg(a[1]))


def cmuli(a, s):
    return (vneg(a[1]), a[0]) if s > 0 else (a[1], vneg(a[0]))


def _snap(x):
    for v in (0.0, 1.0, -1.0):
        if abs(x - v) < 1e-12:
            return v
    return x


def croot(num, den, sgn):
    ang = sgn * 2.0 * math.pi * (num % den) / den
    return _snap(math.cos(ang)), _snap(math.sin(ang))


def cmulc(z, c, s):
    re, im = z
    if s == 0.0:
        return (vmulc(re, c), vmulc(im, c))
    if c == 0.0:
        return (vmulc(im, -s), vmulc(re, s))
    if im is None:
        return (vmulc(re, c), vmulc(re, s))
    if re is None:
        return (vmulc(im, -s), vmulc(im, c))
    if abs(abs(c) - abs(s)) < 1e-12:
        if s / c > 0:
            return (vmulc(vsub(re, im), c), vmulc(vadd(re, im), c))
        return (vmulc(vadd(re, im), c), vmulc(vsub(im, re), c))
    return (vsub(vmulc(re, c), vmulc(im, s)), vadd(vmulc(re, s), vmulc(im, c)))


def dft(xs, sgn):
    n = len(xs)
    if n == 1:
        return list(xs)
    if n == 2:
        return [cadd(xs[0], xs[1]), csub(xs[0], xs[1])]
    U = dft(xs[0::2], sgn)
    Z = dft(xs[1::4], sgn)
    Zp = dft(xs[3::4], sgn)
    out = [None] * n
    q = n // 4
    for k in range(q):
        t1 = cmulc(Z[k], *croot(k, n, sgn))
        t2 = cmulc(Zp[k], *croot(3 * k, n, sgn))
        s = cadd(t1, t2)
        d = cmuli(csub(t1, t2), sgn)
        out[k] = cadd(U[k], s)
        out[k + 2 * q] = csub(U[k], s)
        out[k + q] = cadd(U[k + q], d)
        out[k + 3 * q] = csub(U[k + q], d)
    return out


def rdft(xs):
    n = len(xs)
    if n == 1:
        return [(xs[0], None)]
    if n == 2:
        return [(vadd(xs[0], xs[1]), None), (vsub(xs[0], xs[1]), None)]
    E = rdft(xs[0::2])
    O = rdft(xs[1::2])
    out = [None] * (n // 2 + 1)
    for k in range(n // 4 + 1):
        t = cmulc(O[k], *croot(k, n, -1))
        out[k] = cadd(E[k], t)
        if k != n // 4:
            out[n // 2 - k] = conj(csub(E[k], t))
    return out


N = 128
KT = 31
L = N - KT + 1
NB = 84
NQ = 21
BSTR = NB * L
XOFF = 32
XROWS = 2 * BSTR + 32
TROWS = 9 * 8 * 2 * 16


def _slots():
    s = []
    for u in range(9):
        for k2 in range(8):
            if u == 0 and k2 > 4:
                continue
            if u == 8 and k2 > 3:
                continue
            s.append((u, k2))
    return s


SLOTS = _slots()
NS = len(SLOTS)
SIDX = {uk: i for i, uk in enumerate(SLOTS)}
YROWS = NS * 672


def f32(u):
    return pltpu.bitcast(u, jnp.float32)


def u32(v):
    return pltpu.bitcast(v, jnp.uint32)


def fwd_pass1(xs_ref, q, n2):
    base = 2 + q * (8 * L)
    xin = []
    for n1 in range(16):
        u = xs_ref[pl.ds(base + 8 * n1 + n2, 8, stride=L), :]
        xin.append(((f32(u << 16), 1), (f32(u & jnp.uint32(0xFFFF0000)), 1)))
    X1 = dft(xin, -1)
    for u in range(9):
        top = cmulc(X1[u], *croot(n2 * u, N, -1))
        kp = (16 - u) % 16
        bt = conj(cmulc(X1[kp], *croot(n2 * kp - (16 * n2 if u > 0 else 0), N, -1)))
        for ri in range(2):
            r0 = XROWS + ((u * 8 + n2) * 2 + ri) * 16
            xs_ref[pl.ds(r0, 8), :] = u32(vmat(top[ri]))
            xs_ref[pl.ds(r0 + 8, 8), :] = u32(vmat(bt[ri]))


def fwd_pass2(xs_ref, xh_ref, h, q, u):
    rows = pl.ds(pl.multiple_of(q * 16, 16), 16)
    zin = []
    for n2 in range(8):
        r0 = XROWS + ((u * 8 + n2) * 2) * 16
        zin.append(((f32(xs_ref[pl.ds(r0, 16), :]), 1), (f32(xs_ref[pl.ds(r0 + 16, 16), :]), 1)))
    X2 = dft(zin, -1)
    for k2 in range(8):
        if (u, k2) not in SIDX:
            continue
        j = SIDX[u, k2]
        a, b = X2[k2]
        xh_ref[j, 0, h, rows, :] = vmat(a).astype(jnp.bfloat16)
        xh_ref[j, 1, h, rows, :] = vmat(b).astype(jnp.bfloat16)
        xh_ref[j, 2, h, rows, :] = vmat(vadd(a, b)).astype(jnp.bfloat16)


def fwd_column(xs, xh_ref, q):
    for n2 in range(8):
        for h in range(2):
            fwd_pass1(xs[h], q, n2)
    for u in range(9):
        for h in range(2):
            fwd_pass2(xs[h], xh_ref, h, q, u)


def wt_group(w_ref, tw_ref, wh_ref, r, scale):
    x = {}
    for j in range(KT):
        i = KT - 1 - j
        wv = pltpu.bitcast(w_ref[pl.ds(pl.multiple_of(i * 128 + r * 8, 8), 8), :], jnp.bfloat16)
        x[j] = (wv.astype(jnp.float32), 1)
    for rr in range(8):
        Y = rdft([x.get(rr + 8 * m) for m in range(16)])
        for u in range(9):
            t = cmulc(Y[u], *croot(rr * u, N, -1))
            for ri in range(2):
                if t[ri] is not None:
                    tw_ref[pl.ds(((u * 8 + rr) * 2 + ri) * 16, 16), :] = vmat(vmulc(t[ri], scale))
    rows = pl.ds(pl.multiple_of(r * 16, 16), 16)
    for u in range(9):
        def ld(rr, ri):
            if ri == 1 and (u == 0 or rr == 0 and u == 8):
                return None
            return (tw_ref[pl.ds(((u * 8 + rr) * 2 + ri) * 16, 16), :], 1)
        if u == 0:
            X2 = rdft([ld(rr, 0) for rr in range(8)])
        else:
            X2 = dft([(ld(rr, 0), ld(rr, 1)) for rr in range(8)], -1)
        for k2 in range(8):
            if (u, k2) not in SIDX:
                continue
            j = SIDX[u, k2]
            c, d = X2[k2]
            wh_ref[j, 0, rows, :] = vmat(c).astype(jnp.bfloat16)
            wh_ref[j, 1, rows, :] = vmat(vsub(d, c)).astype(jnp.bfloat16)
            wh_ref[j, 2, rows, :] = vmat(vadd(c, d)).astype(jnp.bfloat16)


def mm_slot(xh_u, wh_u, y_ref, j):
    def lhs(t):
        return jnp.concatenate([pltpu.bitcast(xh_u[j, t, h], jnp.bfloat16) for h in range(2)], axis=1)

    def rhs(t):
        return pltpu.bitcast(wh_u[j, t], jnp.bfloat16)
    k1 = jnp.dot(lhs(2), rhs(0), preferred_element_type=jnp.float32)
    k2 = jnp.dot(lhs(0), rhs(1), preferred_element_type=jnp.float32)
    k3 = jnp.dot(lhs(1), rhs(2), preferred_element_type=jnp.float32)
    base = pl.multiple_of(j * 672, 16) if not isinstance(j, int) else j * 672
    y_ref[pl.ds(base, 336), :] = u32(k1 - k3)
    y_ref[pl.ds(base + 336, 336), :] = u32(k1 + k2)


def yloc(f):
    f2, f1 = f % 16, f // 16
    if 1 <= f2 <= 7:
        return SIDX[f2, f1], 0
    if f2 >= 9:
        return SIDX[16 - f2, 7 - f1], 1
    if f2 == 0:
        return (SIDX[0, f1], 0) if f1 <= 4 else (SIDX[0, 8 - f1], 1)
    return (SIDX[8, f1], 0) if f1 <= 3 else (SIDX[8, 7 - f1], 1)


def ifft_passA(y_ref, qrow, f2):
    locs = [yloc(16 * f1 + f2) for f1 in range(8)]
    yin = []
    for (j, tb) in locs:
        r0 = qrow + (j * 672 + 8 * tb)
        re = (f32(y_ref[pl.ds(r0, 8), :]), 1)
        im = (f32(y_ref[pl.ds(r0 + 336, 8), :]), -1 if tb else 1)
        yin.append((re, im))
    A = dft(yin, 1)
    for k1 in range(8):
        t = cmulc(A[k1], *croot(f2 * k1, N, 1))
        j, tb = locs[k1]
        r0 = qrow + (j * 672 + 8 * tb)
        y_ref[pl.ds(r0, 8), :] = u32(vmat(t[0]))
        y_ref[pl.ds(r0 + 336, 8), :] = u32(vmat(t[1]))


def ifft_passB(y_ref, s_ref, q, qrow, k1, is_gate):
    tin = []
    for f2 in range(16):
        j, tb = yloc(16 * k1 + f2)
        r0 = qrow + (j * 672 + 8 * tb)
        tin.append(((f32(y_ref[pl.ds(r0, 8), :]), 1), (f32(y_ref[pl.ds(r0 + 336, 8), :]), 1)))
    Y = dft(tin, 1)
    for k2 in range(16):
        n = k1 + 8 * k2
        if n < KT - 1:
            continue
        m = n - (KT - 1)
        for part in range(2):
            v = jnp.tanh(vmat(Y[k2][part]))
            idx = pl.ds(q * (16 * L) + (2 * m + part), 8, stride=2 * L)
            if is_gate:
                v = s_ref[idx, :] * (0.5 * v + 0.5)
            s_ref[idx, :] = v


def ifft_column(y_ref, s_ref, q, is_gate):
    qrow = pl.multiple_of(q * 16, 16)
    for f2 in range(16):
        ifft_passA(y_ref, qrow, f2)
    for k1 in range(8):
        ifft_passB(y_ref, s_ref, q, qrow, k1, is_gate)


def kern(x_hbm, w_hbm, o_hbm, y0, y1, xh_ref, wh_ref, s_ref, ws_ref, tw_ref, ob_ref, sem, wsem, osem):
    ys = (y0, y1)
    xu = x_hbm.bitcast(jnp.uint32)
    wu = w_hbm.bitcast(jnp.uint32)
    xcp = [pltpu.make_async_copy(xu.at[b, :, pl.ds(128 * h, 128)], ys[h].at[pl.ds(XOFF + b * BSTR, 8000)], sem.at[2 * b + h])
           for b in range(2) for h in range(2)]
    lane0 = (0, 256, 128, 384)

    def wcp(c):
        return pltpu.make_async_copy(wu.at[:, :, pl.ds(lane0[c], 128)], ws_ref, wsem.at[0])
    wcp(0).start()
    for c in xcp:
        c.start()
    for h in range(2):
        ys[h][pl.ds(0, 32), :] = jnp.zeros((32, 128), jnp.uint32)
        ys[h][pl.ds(8032, 232), :] = jnp.zeros((232, 128), jnp.uint32)
        ys[h][pl.ds(16264, 232), :] = jnp.zeros((232, 128), jnp.uint32)
    for c in xcp:
        c.wait()

    def fwd_body(q, _):
        fwd_column(ys, xh_ref, q)
        return 0
    jax.lax.fori_loop(0, NQ, fwd_body, 0)

    xh_u = xh_ref.bitcast(jnp.uint32)
    wh_u = wh_ref.bitcast(jnp.uint32)
    ws2 = ws_ref
    for c in range(4):
        is_gate = (c % 2 == 1)
        wcp(c).wait()

        def wt_body(r, _):
            wt_group_3d(ws2, tw_ref, wh_ref, r, (0.5 if is_gate else 1.0) / N)
            return 0
        jax.lax.fori_loop(0, 16, wt_body, 0)
        if c < 3:
            wcp(c + 1).start()
        y = ys[c % 2]

        def mm_body(i, _):
            for s in range(3):
                mm_slot(xh_u, wh_u, y, 3 * i + s)
            return 0
        jax.lax.fori_loop(0, NQ, mm_body, 0)
        for j in range(3 * NQ, NS):
            mm_slot(xh_u, wh_u, y, j)

        def ifft_body(q, _):
            ifft_column(y, s_ref, q, is_gate)
            return 0
        jax.lax.fori_loop(0, NQ, ifft_body, 0)
        if is_gate:
            hh = c // 2
            if hh == 1:
                for b in range(2):
                    pltpu.make_async_copy(ob_ref.at[pl.ds(2 * BSTR * b, 16000)], o_hbm.at[b, :, pl.ds(0, 128)], osem.at[b]).wait()

            def cv_body(i, _):
                rows = pl.ds(pl.multiple_of(i * 112, 16), 112)
                ob_ref[rows, :] = s_ref[rows, :].astype(jnp.bfloat16)
                return 0
            jax.lax.fori_loop(0, 2 * 2 * BSTR // 112, cv_body, 0)
            for b in range(2):
                cp = pltpu.make_async_copy(ob_ref.at[pl.ds(2 * BSTR * b, 16000)], o_hbm.at[b, :, pl.ds(128 * hh, 128)], osem.at[b])
                cp.start()
            if hh == 1:
                for b in range(2):
                    pltpu.make_async_copy(ob_ref.at[pl.ds(2 * BSTR * b, 16000)], o_hbm.at[b, :, pl.ds(128, 128)], osem.at[b]).wait()


def wt_group_3d(ws, tw_ref, wh_ref, r, scale):
    class _V:
        def __getitem__(self, idx):
            raise NotImplementedError
    x = {}
    for j in range(KT):
        i = KT - 1 - j
        wv = pltpu.bitcast(ws[i, pl.ds(pl.multiple_of(r * 8, 8), 8), :], jnp.bfloat16)
        x[j] = (wv.astype(jnp.float32), 1)
    for rr in range(8):
        Y = rdft([x.get(rr + 8 * m) for m in range(16)])
        for u in range(9):
            t = cmulc(Y[u], *croot(rr * u, N, -1))
            for ri in range(2):
                if t[ri] is not None:
                    tw_ref[pl.ds(((u * 8 + rr) * 2 + ri) * 16, 16), :] = vmat(vmulc(t[ri], scale))
    rows = pl.ds(pl.multiple_of(r * 16, 16), 16)
    for u in range(9):
        def ld(rr, ri):
            if ri == 1 and (u == 0 or (rr == 0 and u == 8)):
                return None
            return (tw_ref[pl.ds(((u * 8 + rr) * 2 + ri) * 16, 16), :], 1)
        if u == 0:
            X2 = rdft([ld(rr, 0) for rr in range(8)])
        else:
            X2 = dft([(ld(rr, 0), ld(rr, 1)) for rr in range(8)], -1)
        for k2 in range(8):
            if (u, k2) not in SIDX:
                continue
            j = SIDX[u, k2]
            c, d = X2[k2]
            wh_ref[j, 0, rows, :] = vmat(c).astype(jnp.bfloat16)
            wh_ref[j, 1, rows, :] = vmat(vsub(d, c)).astype(jnp.bfloat16) if d is not None else (-vmat(c)).astype(jnp.bfloat16)
            wh_ref[j, 2, rows, :] = vmat(vadd(c, d)).astype(jnp.bfloat16)


@jax.jit
def pallas_standalone__autoregressive_conv_wavernn__speech_kernel(
    x: jax.Array,
    w: jax.Array,
):
    return pl.pallas_call(
        kern,
        in_specs=[pl.BlockSpec(memory_space=pl.ANY), pl.BlockSpec(memory_space=pl.ANY)],
        out_specs=pl.BlockSpec(memory_space=pl.ANY),
        out_shape=jax.ShapeDtypeStruct(x.shape, x.dtype),
        scratch_shapes=[
            pltpu.VMEM((YROWS, 128), jnp.uint32), pltpu.VMEM((YROWS, 128), jnp.uint32),
            pltpu.VMEM((NS, 3, 2, 336, 128), jnp.bfloat16),
            pltpu.VMEM((NS, 3, 256, 128), jnp.bfloat16),
            pltpu.VMEM((4 * BSTR, 128), jnp.float32),
            pltpu.VMEM((31, 128, 128), jnp.uint32),
            pltpu.VMEM((9 * 8 * 2 * 16, 128), jnp.float32),
            pltpu.VMEM((4 * BSTR, 128), jnp.bfloat16),
            pltpu.SemaphoreType.DMA((4,)), pltpu.SemaphoreType.DMA((1,)), pltpu.SemaphoreType.DMA((2,)),
        ],
        compiler_params=pltpu.CompilerParams(vmem_limit_bytes=127 * 1024 * 1024),
    )(x, w)
```

```python
import math
import numpy as np
import jax
import jax.numpy as jnp
from jax.experimental import pallas as pl
from jax.experimental.pallas import tpu as pltpu

def vneg(a):
    return None if a is None else (a[0], -a[1])


def vadd(a, b):
    if a is None:
        return b
    if b is None:
        return a
    if a[1] > 0 and b[1] > 0:
        return (a[0] + b[0], 1)
    if a[1] > 0 and b[1] < 0:
        return (a[0] - b[0], 1)
    if a[1] < 0 and b[1] > 0:
        return (b[0] - a[0], 1)
    return (a[0] + b[0], -1)


def vsub(a, b):
    return vadd(a, vneg(b))


def vmulc(a, c):
    if a is None or c == 0.0:
        return None
    if c == 1.0:
        return a
    if c == -1.0:
        return vneg(a)
    return (a[0] * float(np.float32(c * a[1])), 1)


def vmat(a):
    return a[0] if a[1] > 0 else -a[0]


def cadd(a, b):
    return (vadd(a[0], b[0]), vadd(a[1], b[1]))


def csub(a, b):
    return (vsub(a[0], b[0]), vsub(a[1], b[1]))


def conj(a):
    return (a[0], vneg(a[1]))


def cmuli(a, s):
    return (vneg(a[1]), a[0]) if s > 0 else (a[1], vneg(a[0]))


def _snap(x):
    for v in (0.0, 1.0, -1.0):
        if abs(x - v) < 1e-12:
            return v
    return x


def croot(num, den, sgn):
    ang = sgn * 2.0 * math.pi * (num % den) / den
    return _snap(math.cos(ang)), _snap(math.sin(ang))


def cmulc(z, c, s):
    re, im = z
    if s == 0.0:
        return (vmulc(re, c), vmulc(im, c))
    if c == 0.0:
        return (vmulc(im, -s), vmulc(re, s))
    if im is None:
        return (vmulc(re, c), vmulc(re, s))
    if re is None:
        return (vmulc(im, -s), vmulc(im, c))
    if abs(abs(c) - abs(s)) < 1e-12:
        if s / c > 0:
            return (vmulc(vsub(re, im), c), vmulc(vadd(re, im), c))
        return (vmulc(vadd(re, im), c), vmulc(vsub(im, re), c))
    return (vsub(vmulc(re, c), vmulc(im, s)), vadd(vmulc(re, s), vmulc(im, c)))


def dft(xs, sgn):
    n = len(xs)
    if n == 1:
        return list(xs)
    if n == 2:
        return [cadd(xs[0], xs[1]), csub(xs[0], xs[1])]
    U = dft(xs[0::2], sgn)
    Z = dft(xs[1::4], sgn)
    Zp = dft(xs[3::4], sgn)
    out = [None] * n
    q = n // 4
    for k in range(q):
        t1 = cmulc(Z[k], *croot(k, n, sgn))
        t2 = cmulc(Zp[k], *croot(3 * k, n, sgn))
        s = cadd(t1, t2)
        d = cmuli(csub(t1, t2), sgn)
        out[k] = cadd(U[k], s)
        out[k + 2 * q] = csub(U[k], s)
        out[k + q] = cadd(U[k + q], d)
        out[k + 3 * q] = csub(U[k + q], d)
    return out


def rdft(xs):
    n = len(xs)
    if n == 1:
        return [(xs[0], None)]
    if n == 2:
        return [(vadd(xs[0], xs[1]), None), (vsub(xs[0], xs[1]), None)]
    E = rdft(xs[0::2])
    O = rdft(xs[1::2])
    out = [None] * (n // 2 + 1)
    for k in range(n // 4 + 1):
        t = cmulc(O[k], *croot(k, n, -1))
        out[k] = cadd(E[k], t)
        if k != n // 4:
            out[n // 2 - k] = conj(csub(E[k], t))
    return out


N = 128
KT = 31
L = N - KT + 1
NB = 84
NQ = 21
BSTR = NB * L
XOFF = 32
XROWS = 2 * BSTR + 32
TROWS = 9 * 8 * 2 * 16
XPIECE = 2000


def _slots():
    s = []
    for u in range(9):
        for k2 in range(8):
            if u == 0 and (k2 == 0 or k2 >= 4):
                continue
            if u == 8 and k2 > 3:
                continue
            s.append((u, k2))
    return s


SLOTS = _slots()
NG = len(SLOTS)
SP = NG
NS = NG + 1
SIDX = {uk: i for i, uk in enumerate(SLOTS)}
YROWS = NS * 672
TWROWS = 9 * 8 * 2 * 16


def f32(u):
    return pltpu.bitcast(u, jnp.float32)


def u32(v):
    return pltpu.bitcast(v, jnp.uint32)


def bf(v):
    return v.astype(jnp.bfloat16)


def fwd_pass1(xs_ref, q, n2):
    base = 2 + q * (8 * L)
    xin = []
    for n1 in range(16):
        u = xs_ref[pl.ds(base + 8 * n1 + n2, 8, stride=L), :]
        xin.append(((f32(u << 16), 1), (f32(u & jnp.uint32(0xFFFF0000)), 1)))
    X1 = dft(xin, -1)
    for u in range(9):
        top = cmulc(X1[u], *croot(n2 * u, N, -1))
        kp = (16 - u) % 16
        bt = conj(cmulc(X1[kp], *croot(n2 * kp - (16 * n2 if u > 0 else 0), N, -1)))
        for ri in range(2):
            r0 = XROWS + ((u * 8 + n2) * 2 + ri) * 16
            xs_ref[pl.ds(r0, 8), :] = u32(vmat(top[ri]))
            xs_ref[pl.ds(r0 + 8, 8), :] = u32(vmat(bt[ri]))


def fwd_pass2(xs_ref, xh_ref, h, q, u):
    rows = pl.ds(pl.multiple_of(q * 16, 16), 16)
    zin = []
    for n2 in range(8):
        r0 = XROWS + ((u * 8 + n2) * 2) * 16
        zin.append(((f32(xs_ref[pl.ds(r0, 16), :]), 1), (f32(xs_ref[pl.ds(r0 + 16, 16), :]), 1)))
    X2 = dft(zin, -1)
    for k2 in range(8):
        if u == 0 and k2 in (0, 4):
            a, b = vmat(X2[k2][0]), vmat(X2[k2][1])
            xh_ref[SP, k2 // 4, h, rows, :] = bf(jnp.concatenate([a[0:8], b[0:8]], axis=0))
        if (u, k2) not in SIDX:
            continue
        j = SIDX[u, k2]
        a, b = X2[k2]
        xh_ref[j, 0, h, rows, :] = bf(vmat(a))
        xh_ref[j, 1, h, rows, :] = bf(vmat(b))
        xh_ref[j, 2, h, rows, :] = bf(vmat(vadd(a, b)))


def fwd_column(xs, xh_ref, q):
    for n2 in range(8):
        for h in range(2):
            fwd_pass1(xs[h], q, n2)
    for u in range(9):
        for h in range(2):
            fwd_pass2(xs[h], xh_ref, h, q, u)


def _wt_nonzero():
    class _P:
        def __add__(self, o): return self
        __sub__ = __mul__ = __radd__ = __rsub__ = __rmul__ = __add__
    nz = {}
    for rr in range(8):
        Y = rdft([(_P(), 1) if rr + 8 * m < KT else None for m in range(16)])
        for u in range(9):
            t = cmulc(Y[u], *croot(rr * u, N, -1))
            for ri in range(2):
                nz[rr, u, ri] = t[ri] is not None
    return nz


WT_NONZERO = _wt_nonzero()


def wt_pieces(ws, tw_ref, wh_ref, r, scale, g1=2, g2=2):
    r8 = pl.ds(pl.multiple_of(r * 8, 8), 8)
    rows = pl.ds(pl.multiple_of(r * 16, 16), 16)

    def tap(j):
        if j >= KT:
            return None
        wv = pltpu.bitcast(ws[KT - 1 - j, r8, :], jnp.bfloat16)
        return (wv.astype(jnp.float32) * float(scale), 1)

    def p1(rr):
        Y = rdft([tap(rr + 8 * m) for m in range(16)])
        for u in range(9):
            t = cmulc(Y[u], *croot(rr * u, N, -1))
            for ri in range(2):
                if t[ri] is not None:
                    tw_ref[pl.ds(((u * 8 + rr) * 2 + ri) * 16, 16), :] = vmat(t[ri])

    def p2(u):
        def ld(rr, ri):
            if not WT_NONZERO[rr, u, ri]:
                return None
            return (tw_ref[pl.ds(((u * 8 + rr) * 2 + ri) * 16, 16), :], 1)
        if u == 0:
            X2 = rdft([ld(rr, 0) for rr in range(8)])
        else:
            X2 = dft([(ld(rr, 0), ld(rr, 1)) for rr in range(8)], -1)
        for k2 in range(8):
            if u == 0 and k2 in (0, 4):
                wh_ref[SP, k2 // 4, rows, :] = bf(vmat(X2[k2][0]))
            if (u, k2) not in SIDX:
                continue
            j = SIDX[u, k2]
            c, d = X2[k2]
            wh_ref[j, 0, rows, :] = bf(vmat(c))
            wh_ref[j, 1, rows, :] = bf(vmat(vsub(d, c)))
            wh_ref[j, 2, rows, :] = bf(vmat(vadd(c, d)))

    pieces = []
    for r0 in range(0, 8, g1):
        pieces.append(lambda r0=r0: [p1(rr) for rr in range(r0, r0 + g1)])
    us = [1, 2, 3, 4, 5, 6, 7, 0, 8]
    for i in range(0, 9, g2):
        pieces.append(lambda i=i: [p2(u) for u in us[i:i + g2]])
    return pieces


def _lhs(xh_u, j, t):
    return jnp.concatenate([pltpu.bitcast(xh_u[j, t, h], jnp.bfloat16) for h in range(2)], axis=1)


def _rhs(wh_u, j, t):
    return pltpu.bitcast(wh_u[j, t], jnp.bfloat16)


def _dot(a, b):
    return jnp.dot(a, b, preferred_element_type=jnp.float32)


def mm_slot(xh_u, wh_u, y_ref, j, acc=None, step=1, temp=True):
    if temp:
        base = pl.multiple_of(j * 672, 16) if not isinstance(j, int) else j * 672
        rre, rim = pl.ds(base, 336), pl.ds(base + 336, 336)
        k1 = _dot(_lhs(xh_u, j, 2), _rhs(wh_u, j, 0))
        y_ref[rre, :] = u32(k1)
        k2 = _dot(_lhs(xh_u, j, 0), _rhs(wh_u, j, 1))
        im = f32(y_ref[rre, :]) + k2
        y_ref[rim, :] = u32(im)
        k3 = _dot(_lhs(xh_u, j, 1), _rhs(wh_u, j, 2))
        re = f32(y_ref[rre, :]) - k3
        y_ref[rre, :] = u32(re)
        if acc is not None:
            for v in (k1, im, re):
                for i in range(0, 21, step):
                    for hh in (0, 21):
                        acc[0] = acc[0] + v[8 * (i + hh):8 * (i + hh) + 8]
        return [k[r:r + 8] for k in (k1, k2, k3) for r in (0, 40, 80, 120, 160)]
    k1 = _dot(_lhs(xh_u, j, 2), _rhs(wh_u, j, 0))
    k2 = _dot(_lhs(xh_u, j, 0), _rhs(wh_u, j, 1))
    k3 = _dot(_lhs(xh_u, j, 1), _rhs(wh_u, j, 2))
    base = pl.multiple_of(j * 672, 16) if not isinstance(j, int) else j * 672
    y_ref[pl.ds(base, 336), :] = u32(k1 - k3)
    y_ref[pl.ds(base + 336, 336), :] = u32(k1 + k2)
    if acc is not None:
        im = k1 + k2
        re = k1 - k3
        for v in (im, re):
            for i in range(0, 21, step):
                for hh in (0, 21):
                    acc[0] = acc[0] + v[8 * (i + hh):8 * (i + hh) + 8]
    return [k[r:r + 8] for k in (k1, k2, k3) for r in (0, 40, 80, 120, 160)]


def mm_special(xh_u, wh_u, y_ref):
    for t in range(2):
        y_ref[pl.ds(SP * 672 + 336 * t, 336), :] = u32(_dot(_lhs(xh_u, SP, t), _rhs(wh_u, SP, t)))


def yrows(f):
    f2, f1 = f % 16, f // 16
    if f == 0:
        return SP * 672, SP * 672 + 8, 1
    if f == 64:
        return SP * 672 + 336, SP * 672 + 344, 1
    if 1 <= f2 <= 7:
        j, tb = SIDX[f2, f1], 0
    elif f2 >= 9:
        j, tb = SIDX[16 - f2, 7 - f1], 1
    elif f2 == 0:
        j, tb = (SIDX[0, f1], 0) if f1 < 4 else (SIDX[0, 8 - f1], 1)
    else:
        j, tb = (SIDX[8, f1], 0) if f1 <= 3 else (SIDX[8, 7 - f1], 1)
    r = j * 672 + 8 * tb
    return r, r + 336, (-1 if tb else 1)


def ifft_passA(y_ref, qrow, f2):
    locs = [yrows(16 * f1 + f2) for f1 in range(8)]
    yin = []
    for (rr, ri, sg) in locs:
        yin.append(((f32(y_ref[pl.ds(qrow + rr, 8), :]), 1), (f32(y_ref[pl.ds(qrow + ri, 8), :]), sg)))
    A = dft(yin, 1)
    for k1 in range(8):
        t = cmulc(A[k1], *croot(f2 * k1, N, 1))
        rr, ri, _ = locs[k1]
        y_ref[pl.ds(qrow + rr, 8), :] = u32(vmat(t[0]))
        y_ref[pl.ds(qrow + ri, 8), :] = u32(vmat(t[1]))


def _ld(y_ref, r):
    return (f32(y_ref[pl.ds(r, 8), :]), 1)


def ifft_emit(s_ref, st_ref, srow, k1, k2, y, is_gate):
    n = k1 + 8 * k2
    if n < KT - 1:
        return
    m = n - (KT - 1)
    v = [jnp.tanh(vmat(y[part])) for part in range(2)]
    idx = pl.ds(srow + 16 * m, 16)
    if is_gate:
        t = s_ref[idx, :].astype(jnp.float32)
        for part in range(2):
            st_ref[pl.ds(2 * m + part, 8, stride=2 * L), :] = t[8 * part:8 * part + 8] * (0.5 * v[part] + 0.5)
    else:
        s_ref[idx, :] = bf(jnp.concatenate(v, axis=0))


def ifft_passB(y_ref, s_ref, st_ref, srow, qrow, k1, is_gate):
    tin = []
    for f2 in range(16):
        rr, ri, _ = yrows(16 * k1 + f2)
        tin.append((_ld(y_ref, qrow + rr), _ld(y_ref, qrow + ri)))
    Y = dft(tin, 1)
    for k2 in range(16):
        ifft_emit(s_ref, st_ref, srow, k1, k2, Y[k2], is_gate)


def ifft_passB1(y_ref, qrow, k1):
    locs = [yrows(16 * k1 + f2) for f2 in range(1, 16, 2)]
    O = dft([(_ld(y_ref, qrow + rr), _ld(y_ref, qrow + ri)) for rr, ri, _ in locs], 1)
    for k in range(8):
        t = cmulc(O[k], *croot(k, 16, 1))
        rr, ri, _ = locs[k]
        y_ref[pl.ds(qrow + rr, 8), :] = u32(vmat(t[0]))
        y_ref[pl.ds(qrow + ri, 8), :] = u32(vmat(t[1]))


def ifft_passB2(y_ref, s_ref, st_ref, srow, qrow, k1, is_gate):
    le = [yrows(16 * k1 + f2) for f2 in range(0, 16, 2)]
    lo = [yrows(16 * k1 + f2) for f2 in range(1, 16, 2)]
    E = dft([(_ld(y_ref, qrow + rr), _ld(y_ref, qrow + ri)) for rr, ri, _ in le], 1)
    for k in range(8):
        rr, ri, _ = lo[k]
        o = (_ld(y_ref, qrow + rr), _ld(y_ref, qrow + ri))
        if k1 + 8 * k >= KT - 1:
            ifft_emit(s_ref, st_ref, srow, k1, k, cadd(E[k], o), is_gate)
        ifft_emit(s_ref, st_ref, srow, k1, k + 8, csub(E[k], o), is_gate)


def ifft_sp(y_ref, s_ref, st_ref, ob_ref, q2, is_gate, doA, doB1, doB2):
    base = pl.multiple_of(q2 * 16, 16) if not isinstance(q2, int) else q2 * 16
    srow = pl.multiple_of(q2 * (16 * L), 16) if not isinstance(q2, int) else q2 * 16 * L
    out = []
    if doA:
        out += [lambda f2=f2: ifft_passA(y_ref, base + 32, f2) for f2 in range(16)]
    if doB1:
        out += [lambda k1=k1: ifft_passB1(y_ref, base + 16, k1) for k1 in range(8)]
    if doB2:
        out += [lambda k1=k1: ifft_passB2(y_ref, s_ref, st_ref, srow, base, k1, is_gate) for k1 in range(8)]
        if is_gate:
            def cv():
                for i in range(L):
                    ob_ref[pl.ds(srow + 16 * i, 16), :] = bf(st_ref[pl.ds(16 * i, 16), :])
            out.append(cv)
    return out


def ifft_pieces(y_ref, s_ref, st_ref, ob_ref, q, is_gate, ga, gb):
    qrow = pl.multiple_of(q * 16, 16)
    srow = pl.multiple_of(q * (16 * L), 16)
    pieces = []
    for f0 in range(0, 16, ga):
        def pa(f0=f0):
            for f2 in range(f0, f0 + ga):
                ifft_passA(y_ref, qrow, f2)
        pieces.append(pa)
    if gb == 0:
        for k1 in range(8):
            pieces.append(lambda k1=k1: ifft_passB1(y_ref, qrow, k1))
            pieces.append(lambda k1=k1: ifft_passB2(y_ref, s_ref, st_ref, srow, qrow, k1, is_gate))
        gb = 99
    for k0 in range(0, 8 if gb != 99 else 0, gb):
        def pb(k0=k0):
            for k1 in range(k0, k0 + gb):
                ifft_passB(y_ref, s_ref, st_ref, srow, qrow, k1, is_gate)
        pieces.append(pb)
    if is_gate:
        def cv():
            for i in range(L):
                ob_ref[pl.ds(srow + 16 * i, 16), :] = bf(st_ref[pl.ds(16 * i, 16), :])
        pieces.append(cv)
    return pieces


LANE0 = (0, 256, 128, 384)
RT = 16 * L
VB = 2 * BSTR


def make_kern(pace=True, ga=2, gb=1, g1=2, g2=2, lead=1, mmfirst=True, chain=0, temp=True, upto=99, sp=False, sporder=0, p2=None, p2w=None):
  def kern(x_hbm, w_hbm, o_hbm, y0, y1, xh_ref, wh0, wh1, s_ref, st_ref, ws_ref, tw_ref, ob_ref, z_ref, xsem, wsem, osem):
    ys = (y0, y1)
    whs = (wh0, wh1)
    xu = x_hbm.bitcast(jnp.uint32)
    wu = w_hbm.bitcast(jnp.uint32)

    def xcp(p, h):
        b, i = divmod(p, 4)
        return pltpu.make_async_copy(xu.at[b, pl.ds(XPIECE * i, XPIECE), pl.ds(128 * h, 128)],
                                     ys[h].at[pl.ds(XOFF + b * BSTR + XPIECE * i, XPIECE)], xsem.at[2 * p + h])

    def wcp(c):
        return pltpu.make_async_copy(wu.at[:, :, pl.ds(LANE0[c], 128)], ws_ref.at[c % 2], wsem.at[c % 2])

    z_ref[0] = 0
    wcp(0).start()
    XAHEAD = 3
    for p in range(XAHEAD):
        for h in range(2):
            xcp(p, h).start()
    for h in range(2):
        ys[h][pl.ds(0, 32), :] = jnp.zeros((32, 128), jnp.uint32)
        ys[h][pl.ds(8032, 232), :] = jnp.zeros((232, 128), jnp.uint32)
        ys[h][pl.ds(16264, 232), :] = jnp.zeros((232, 128), jnp.uint32)

    def scale(c):
        return (0.5 if c % 2 == 1 else 1.0) / N

    wcp(0).wait()

    def wt0_body(r, _):
        for p in wt_pieces(ws_ref.at[0], tw_ref, whs[0], r, scale(0)):
            p()
        return 0
    jax.lax.fori_loop(0, 16, wt0_body, 0)

    first_q = {}
    for p in range(8):
        b, i = divmod(p, 4)
        st = XOFF + b * BSTR + XPIECE * i
        first_q[p] = min(q for q in range(NQ) if 8 * L * q + 2 + 7 * L + N > st)

    def fwd_body(q, _):
        for p in range(8):
            @pl.when(q == first_q[p])
            def _():
                for h in range(2):
                    xcp(p, h).wait()
                if p + XAHEAD < 8:
                    for h in range(2):
                        xcp(p + XAHEAD, h).start()
                if p == 5:
                    wcp(1).start()
                if p == 7:
                    wcp(2).start()
        fwd_column(ys, xh_ref, q)
        return 0
    jax.lax.fori_loop(0, NQ, fwd_body, 0)

    xh_u = xh_ref.bitcast(jnp.uint32)

    def ocp(hh, b, t0, n, k):
        return pltpu.make_async_copy(ob_ref.at[pl.ds(VB * b + t0, n)], o_hbm.at[b, pl.ds(t0, n), pl.ds(128 * hh, 128)], osem.at[k])

    def paced2(pieces, npaced, tokens, ref, zero_row, lead, tstep, t0=0):
        for k, p in enumerate(pieces):
            if tokens and lead <= k < npaced:
                tk = tokens[min(t0 + (k - lead) * tstep, len(tokens) - 1)]
                ref[pl.ds(zero_row, 8), :] = tk if ref.dtype == jnp.float32 else u32(tk)
            p()

    def paced(pieces, tokens, ref, zero_row, lead):
        n = len(pieces)
        for k, p in enumerate(pieces):
            if pace and tokens and k >= lead:
                tk = tokens[((k - lead) * len(tokens)) // (n - lead + 1)]
                ref[pl.ds(zero_row, 8), :] = tk if ref.dtype == jnp.float32 else u32(tk)
            p()

    def phase(c_mm, c_if, c_wt, ranges):
        is_gate = c_if is not None and c_if % 2 == 1
        if c_mm is not None:
            wh_u = whs[c_mm % 2].bitcast(jnp.uint32)
            mm_special(xh_u, wh_u, ys[c_mm % 2])
        if c_wt is not None:
            wcp(c_wt).wait()
        if c_if is not None and sp:
            yif = ys[c_if % 2]
            for col in range(2):
                for f2 in range(16):
                    ifft_passA(yif, 16 * col, f2)
            for k1 in range(8):
                ifft_passB1(yif, 0, k1)

        def body(q, with_wt, doA=True, doB1=True):
            tokens = []
            if c_mm is not None:
                acc = [jnp.zeros((8, 128), jnp.float32)] if chain and (c_if is not None or with_wt) else None
                for s in range(3):
                    tokens += mm_slot(xh_u, wh_u, ys[c_mm % 2], 3 * q + s, acc, max(chain, 1), temp)
                if acc is not None:
                    ys[c_mm % 2][pl.ds(YROWS, 8), :] = u32(acc[0])
            z = z_ref[0]
            if c_if is not None and sp:
                pcs = ifft_sp(ys[c_if % 2], s_ref, st_ref, ob_ref, q, is_gate, doA, doB1, True)
                if sporder == 1:
                    pcs = pcs[::-1]
                for p in pcs:
                    p()
            elif c_if is not None and p2 is not None:
                yif = ys[c_if % 2]
                paced2(ifft_pieces(yif, s_ref, st_ref, ob_ref, q, is_gate, ga, gb), p2[0], tokens, yif,
                       pl.multiple_of(YROWS + z, 8), p2[1], p2[2])
            elif c_if is not None:
                yif = ys[c_if % 2]
                paced(ifft_pieces(yif, s_ref, st_ref, ob_ref, q, is_gate, ga, gb), tokens, yif,
                      pl.multiple_of(YROWS + z, 8), lead)
            if with_wt and p2w is not None:
                paced2(wt_pieces(ws_ref.at[c_wt % 2], tw_ref, whs[c_wt % 2], q, scale(c_wt), g1, g2), p2w[0], tokens, tw_ref,
                       pl.multiple_of(TWROWS + z, 8), p2w[1], p2w[2])
            elif with_wt:
                paced(wt_pieces(ws_ref.at[c_wt % 2], tw_ref, whs[c_wt % 2], q, scale(c_wt), g1, g2), tokens, tw_ref,
                      pl.multiple_of(TWROWS + z, 8), lead)

        for (q0, q1, after) in ranges:
            with_wt = c_wt is not None and q1 <= 16
            if sp and c_if is not None and q1 == NQ:
                jax.lax.fori_loop(q0, NQ - 2, lambda q, _: (body(q, with_wt), 0)[1], 0)
                body(NQ - 2, False, False, True)
                body(NQ - 1, False, False, False)
            else:
                jax.lax.fori_loop(q0, q1, lambda q, _: (body(q, with_wt), 0)[1], 0)
            if after is not None:
                after()

    def nop():
        pass

    def out0_a():
        ocp(0, 0, 0, 16000, 0).start()
        ocp(0, 1, 0, 16 * RT - VB, 1).start()

    def out0_b():
        ocp(0, 1, 16 * RT - VB, 16000 - (16 * RT - VB), 2).start()

    def out0_wait():
        ocp(0, 0, 0, 16000, 0).wait()
        ocp(0, 1, 0, 16 * RT - VB, 1).wait()
        ocp(0, 1, 16 * RT - VB, 16000 - (16 * RT - VB), 2).wait()

    def out1(k, wait):
        pcs = [(0, 0, 5 * RT), (0, 5 * RT, 16000 - 5 * RT), (1, 0, 15 * RT - VB), (1, 15 * RT - VB, 3 * RT),
               (1, 18 * RT - VB, 16000 - (18 * RT - VB))]
        cp = ocp(1, *pcs[k], 3 + k)
        if wait:
            cp.wait()
        else:
            cp.start()

    def fin():
        z = z_ref[0]
        r = pl.ds(pl.multiple_of(z * 16, 16), 16)
        r8 = pl.ds(pl.multiple_of(z * 8, 8), 8)
        acc = xh_ref[z, z, z, r, :].astype(jnp.float32) + whs[0][z, z, r, :].astype(jnp.float32) + whs[1][z, z, r, :].astype(jnp.float32)
        acc = acc + s_ref[r, :].astype(jnp.float32) + ob_ref[r, :].astype(jnp.float32)
        acc = acc + jnp.concatenate([f32(ys[0][r8, :]), f32(ys[1][r8, :])], axis=0) + st_ref[r, :] + tw_ref[r, :]
        ob_ref[pl.ds(0, 16), :] = bf(acc)
        o = pltpu.make_async_copy(ob_ref.at[pl.ds(0, 16)], o_hbm.at[0, pl.ds(0, 16), pl.ds(0, 128)], osem.at[7])
        o.start(); o.wait()
    if upto == 0:
        wcp(1).wait(); wcp(2).wait(); fin(); return
    phase(0, None, 1, [(0, 16, None), (16, NQ, None)])
    if upto == 1:
        wcp(2).wait(); fin(); return
    wcp(3).start()
    phase(1, 0, 2, [(0, 16, None), (16, NQ, None)])
    if upto == 2:
        wcp(3).wait(); fin(); return
    phase(2, 1, 3, [(0, 16, out0_a), (16, NQ, out0_b)])
    if upto == 3:
        out0_wait(); fin(); return
    phase(3, 2, None, [(0, NQ, None)])
    out0_wait()
    if upto == 4:
        fin(); return

    def tail_body(q, _):
        for p in ifft_pieces(ys[1], s_ref, st_ref, ob_ref, q, True, 16, 8):
            p()
        return 0
    bounds = [0, 5, 11, 15, 18, 21]

    def seg(i, _):
        q0 = jnp.where(i == 0, 0, jnp.where(i == 1, 5, jnp.where(i == 2, 11, jnp.where(i == 3, 15, 18))))
        q1 = jnp.where(i == 0, 5, jnp.where(i == 1, 11, jnp.where(i == 2, 15, jnp.where(i == 3, 18, 21))))
        jax.lax.fori_loop(q0, q1, tail_body, 0)
        for k in range(5):
            @pl.when(i == k)
            def _():
                out1(k, False)
        return 0
    jax.lax.fori_loop(0, 5, seg, 0)
    for k in range(5):
        out1(k, True)
  return kern


@jax.jit
def pallas_standalone__autoregressive_conv_wavernn__speech_kernel(x, w):
    kern = make_kern(**{"ga": 1, "gb": 1, "g1": 1, "g2": 1, "lead": 2})
    flags = None
    return pl.pallas_call(
        kern,
        in_specs=[pl.BlockSpec(memory_space=pl.ANY), pl.BlockSpec(memory_space=pl.ANY)],
        out_specs=pl.BlockSpec(memory_space=pl.ANY),
        out_shape=jax.ShapeDtypeStruct(x.shape, x.dtype),
        scratch_shapes=[
            pltpu.VMEM((YROWS + 8, 128), jnp.uint32), pltpu.VMEM((YROWS + 8, 128), jnp.uint32),
            pltpu.VMEM((NS, 3, 2, 336, 128), jnp.bfloat16),
            pltpu.VMEM((NS, 3, 256, 128), jnp.bfloat16),
            pltpu.VMEM((NS, 3, 256, 128), jnp.bfloat16),
            pltpu.VMEM((2 * VB, 128), jnp.bfloat16),
            pltpu.VMEM((RT, 128), jnp.float32),
            pltpu.VMEM((2, 31, 128, 128), jnp.uint32),
            pltpu.VMEM((TWROWS + 8, 128), jnp.float32),
            pltpu.VMEM((2 * VB, 128), jnp.bfloat16),
            pltpu.SMEM((1,), jnp.int32),
            pltpu.SemaphoreType.DMA((16,)), pltpu.SemaphoreType.DMA((2,)), pltpu.SemaphoreType.DMA((8,)),
        ],
        compiler_params=pltpu.CompilerParams(vmem_limit_bytes=127 * 1024 * 1024, flags=flags),
    )(x, w)
```

```python
import math
import numpy as np
import jax
import jax.numpy as jnp
from jax.experimental import pallas as pl
from jax.experimental.pallas import tpu as pltpu

def vneg(a):
    return None if a is None else (a[0], -a[1])


def vadd(a, b):
    if a is None:
        return b
    if b is None:
        return a
    if a[1] > 0 and b[1] > 0:
        return (a[0] + b[0], 1)
    if a[1] > 0 and b[1] < 0:
        return (a[0] - b[0], 1)
    if a[1] < 0 and b[1] > 0:
        return (b[0] - a[0], 1)
    return (a[0] + b[0], -1)


def vsub(a, b):
    return vadd(a, vneg(b))


def vmulc(a, c):
    if a is None or c == 0.0:
        return None
    if c == 1.0:
        return a
    if c == -1.0:
        return vneg(a)
    return (a[0] * float(np.float32(c * a[1])), 1)


def vmat(a):
    return a[0] if a[1] > 0 else -a[0]


def cadd(a, b):
    return (vadd(a[0], b[0]), vadd(a[1], b[1]))


def csub(a, b):
    return (vsub(a[0], b[0]), vsub(a[1], b[1]))


def conj(a):
    return (a[0], vneg(a[1]))


def cmuli(a, s):
    return (vneg(a[1]), a[0]) if s > 0 else (a[1], vneg(a[0]))


def _snap(x):
    for v in (0.0, 1.0, -1.0):
        if abs(x - v) < 1e-12:
            return v
    return x


def croot(num, den, sgn):
    ang = sgn * 2.0 * math.pi * (num % den) / den
    return _snap(math.cos(ang)), _snap(math.sin(ang))


def cmulc(z, c, s):
    re, im = z
    if s == 0.0:
        return (vmulc(re, c), vmulc(im, c))
    if c == 0.0:
        return (vmulc(im, -s), vmulc(re, s))
    if im is None:
        return (vmulc(re, c), vmulc(re, s))
    if re is None:
        return (vmulc(im, -s), vmulc(im, c))
    if abs(abs(c) - abs(s)) < 1e-12:
        if s / c > 0:
            return (vmulc(vsub(re, im), c), vmulc(vadd(re, im), c))
        return (vmulc(vadd(re, im), c), vmulc(vsub(im, re), c))
    return (vsub(vmulc(re, c), vmulc(im, s)), vadd(vmulc(re, s), vmulc(im, c)))


def dft(xs, sgn):
    n = len(xs)
    if n == 1:
        return list(xs)
    if n == 2:
        return [cadd(xs[0], xs[1]), csub(xs[0], xs[1])]
    U = dft(xs[0::2], sgn)
    Z = dft(xs[1::4], sgn)
    Zp = dft(xs[3::4], sgn)
    out = [None] * n
    q = n // 4
    for k in range(q):
        t1 = cmulc(Z[k], *croot(k, n, sgn))
        t2 = cmulc(Zp[k], *croot(3 * k, n, sgn))
        s = cadd(t1, t2)
        d = cmuli(csub(t1, t2), sgn)
        out[k] = cadd(U[k], s)
        out[k + 2 * q] = csub(U[k], s)
        out[k + q] = cadd(U[k + q], d)
        out[k + 3 * q] = csub(U[k + q], d)
    return out


def rdft(xs):
    n = len(xs)
    if n == 1:
        return [(xs[0], None)]
    if n == 2:
        return [(vadd(xs[0], xs[1]), None), (vsub(xs[0], xs[1]), None)]
    E = rdft(xs[0::2])
    O = rdft(xs[1::2])
    out = [None] * (n // 2 + 1)
    for k in range(n // 4 + 1):
        t = cmulc(O[k], *croot(k, n, -1))
        out[k] = cadd(E[k], t)
        if k != n // 4:
            out[n // 2 - k] = conj(csub(E[k], t))
    return out


N = 128
KT = 31
L = N - KT + 1
NB = 84
NQ = 21
BSTR = NB * L
XOFF = 32
XROWS = 2 * BSTR + 32
TROWS = 9 * 8 * 2 * 16
XPIECE = 2000


def _slots():
    s = []
    for u in range(9):
        for k2 in range(8):
            if u == 0 and (k2 == 0 or k2 >= 4):
                continue
            if u == 8 and k2 > 3:
                continue
            s.append((u, k2))
    return s


SLOTS = _slots()
NG = len(SLOTS)
SP = NG
NS = NG + 1
SIDX = {uk: i for i, uk in enumerate(SLOTS)}
TOKEN_ROWS = (0, 40, 80, 120, 160)
YROWS = NS * 672
TWROWS = 9 * 8 * 2 * 16


def f32(u):
    return pltpu.bitcast(u, jnp.float32)


def u32(v):
    return pltpu.bitcast(v, jnp.uint32)


def bf(v):
    return v.astype(jnp.bfloat16)


def fwd_pass1(xs_ref, q, n2):
    base = 2 + q * (8 * L)
    xin = []
    for n1 in range(16):
        u = xs_ref[pl.ds(base + 8 * n1 + n2, 8, stride=L), :]
        xin.append(((f32(u << 16), 1), (f32(u & jnp.uint32(0xFFFF0000)), 1)))
    X1 = dft(xin, -1)
    for u in range(9):
        top = cmulc(X1[u], *croot(n2 * u, N, -1))
        kp = (16 - u) % 16
        bt = conj(cmulc(X1[kp], *croot(n2 * kp - (16 * n2 if u > 0 else 0), N, -1)))
        for ri in range(2):
            r0 = XROWS + ((u * 8 + n2) * 2 + ri) * 16
            xs_ref[pl.ds(r0, 8), :] = u32(vmat(top[ri]))
            xs_ref[pl.ds(r0 + 8, 8), :] = u32(vmat(bt[ri]))


def fwd_pass2(xs_ref, xh_ref, h, q, u):
    rows = pl.ds(pl.multiple_of(q * 16, 16), 16)
    zin = []
    for n2 in range(8):
        r0 = XROWS + ((u * 8 + n2) * 2) * 16
        zin.append(((f32(xs_ref[pl.ds(r0, 16), :]), 1), (f32(xs_ref[pl.ds(r0 + 16, 16), :]), 1)))
    X2 = dft(zin, -1)
    for k2 in range(8):
        if u == 0 and k2 in (0, 4):
            a, b = vmat(X2[k2][0]), vmat(X2[k2][1])
            xh_ref[SP, k2 // 4, h, rows, :] = bf(jnp.concatenate([a[0:8], b[0:8]], axis=0))
        if (u, k2) not in SIDX:
            continue
        j = SIDX[u, k2]
        a, b = X2[k2]
        xh_ref[j, 0, h, rows, :] = bf(vmat(a))
        xh_ref[j, 1, h, rows, :] = bf(vmat(b))
        xh_ref[j, 2, h, rows, :] = bf(vmat(vadd(a, b)))


def fwd_column(xs, xh_ref, q):
    for n2 in range(8):
        for h in range(2):
            fwd_pass1(xs[h], q, n2)
    for u in range(9):
        for h in range(2):
            fwd_pass2(xs[h], xh_ref, h, q, u)


def _wt_nonzero():
    class _P:
        def __add__(self, o): return self
        __sub__ = __mul__ = __radd__ = __rsub__ = __rmul__ = __add__
    nz = {}
    for rr in range(8):
        Y = rdft([(_P(), 1) if rr + 8 * m < KT else None for m in range(16)])
        for u in range(9):
            t = cmulc(Y[u], *croot(rr * u, N, -1))
            for ri in range(2):
                nz[rr, u, ri] = t[ri] is not None
    return nz


WT_NONZERO = _wt_nonzero()


def wt_pieces(ws, tw_ref, wh_ref, r, scale, g1=2, g2=2):
    r8 = pl.ds(pl.multiple_of(r * 8, 8), 8)
    rows = pl.ds(pl.multiple_of(r * 16, 16), 16)

    def tap(j):
        if j >= KT:
            return None
        wv = pltpu.bitcast(ws[KT - 1 - j, r8, :], jnp.bfloat16)
        return (wv.astype(jnp.float32) * float(scale), 1)

    def p1(rr):
        Y = rdft([tap(rr + 8 * m) for m in range(16)])
        for u in range(9):
            t = cmulc(Y[u], *croot(rr * u, N, -1))
            for ri in range(2):
                if t[ri] is not None:
                    tw_ref[pl.ds(((u * 8 + rr) * 2 + ri) * 16, 16), :] = vmat(t[ri])

    def p2(u):
        def ld(rr, ri):
            if not WT_NONZERO[rr, u, ri]:
                return None
            return (tw_ref[pl.ds(((u * 8 + rr) * 2 + ri) * 16, 16), :], 1)
        if u == 0:
            X2 = rdft([ld(rr, 0) for rr in range(8)])
        else:
            X2 = dft([(ld(rr, 0), ld(rr, 1)) for rr in range(8)], -1)
        for k2 in range(8):
            if u == 0 and k2 in (0, 4):
                wh_ref[SP, k2 // 4, rows, :] = bf(vmat(X2[k2][0]))
            if (u, k2) not in SIDX:
                continue
            j = SIDX[u, k2]
            c, d = X2[k2]
            wh_ref[j, 0, rows, :] = bf(vmat(c))
            wh_ref[j, 1, rows, :] = bf(vmat(vsub(d, c)))
            wh_ref[j, 2, rows, :] = bf(vmat(vadd(c, d)))

    pieces = []
    for r0 in range(0, 8, g1):
        pieces.append(lambda r0=r0: [p1(rr) for rr in range(r0, r0 + g1)])
    us = [1, 2, 3, 4, 5, 6, 7, 0, 8]
    for i in range(0, 9, g2):
        pieces.append(lambda i=i: [p2(u) for u in us[i:i + g2]])
    return pieces


def _lhs(xh_u, j, t):
    return jnp.concatenate([pltpu.bitcast(xh_u[j, t, h], jnp.bfloat16) for h in range(2)], axis=1)


def _rhs(wh_u, j, t):
    return pltpu.bitcast(wh_u[j, t], jnp.bfloat16)


def _dot(a, b):
    return jnp.dot(a, b, preferred_element_type=jnp.float32)


def mm_slot(xh_u, wh_u, y_ref, j):
    base = pl.multiple_of(j * 672, 16) if not isinstance(j, int) else j * 672
    rre, rim = pl.ds(base, 336), pl.ds(base + 336, 336)
    k1 = _dot(_lhs(xh_u, j, 2), _rhs(wh_u, j, 0))
    y_ref[rre, :] = u32(k1)
    k2 = _dot(_lhs(xh_u, j, 0), _rhs(wh_u, j, 1))
    y_ref[rim, :] = u32(f32(y_ref[rre, :]) + k2)
    k3 = _dot(_lhs(xh_u, j, 1), _rhs(wh_u, j, 2))
    y_ref[rre, :] = u32(f32(y_ref[rre, :]) - k3)
    return [k[r:r + 8] for k in (k1, k2, k3) for r in TOKEN_ROWS]


def mm_special(xh_u, wh_u, y_ref):
    for t in range(2):
        y_ref[pl.ds(SP * 672 + 336 * t, 336), :] = u32(_dot(_lhs(xh_u, SP, t), _rhs(wh_u, SP, t)))


def yrows(f):
    f2, f1 = f % 16, f // 16
    if f == 0:
        return SP * 672, SP * 672 + 8, 1
    if f == 64:
        return SP * 672 + 336, SP * 672 + 344, 1
    if 1 <= f2 <= 7:
        j, tb = SIDX[f2, f1], 0
    elif f2 >= 9:
        j, tb = SIDX[16 - f2, 7 - f1], 1
    elif f2 == 0:
        j, tb = (SIDX[0, f1], 0) if f1 < 4 else (SIDX[0, 8 - f1], 1)
    else:
        j, tb = (SIDX[8, f1], 0) if f1 <= 3 else (SIDX[8, 7 - f1], 1)
    r = j * 672 + 8 * tb
    return r, r + 336, (-1 if tb else 1)


def ifft_passA(y_ref, qrow, f2):
    locs = [yrows(16 * f1 + f2) for f1 in range(8)]
    yin = []
    for (rr, ri, sg) in locs:
        yin.append(((f32(y_ref[pl.ds(qrow + rr, 8), :]), 1), (f32(y_ref[pl.ds(qrow + ri, 8), :]), sg)))
    A = dft(yin, 1)
    for k1 in range(8):
        t = cmulc(A[k1], *croot(f2 * k1, N, 1))
        rr, ri, _ = locs[k1]
        y_ref[pl.ds(qrow + rr, 8), :] = u32(vmat(t[0]))
        y_ref[pl.ds(qrow + ri, 8), :] = u32(vmat(t[1]))


def _ld(y_ref, r):
    return (f32(y_ref[pl.ds(r, 8), :]), 1)


def ifft_emit(s_ref, st_ref, srow, k1, k2, y, is_gate):
    n = k1 + 8 * k2
    if n < KT - 1:
        return
    m = n - (KT - 1)
    v = [jnp.tanh(vmat(y[part])) for part in range(2)]
    idx = pl.ds(srow + 16 * m, 16)
    if is_gate:
        t = s_ref[idx, :].astype(jnp.float32)
        for part in range(2):
            st_ref[pl.ds(2 * m + part, 8, stride=2 * L), :] = t[8 * part:8 * part + 8] * (0.5 * v[part] + 0.5)
    else:
        s_ref[idx, :] = bf(jnp.concatenate(v, axis=0))


def ifft_passB(y_ref, s_ref, st_ref, srow, qrow, k1, is_gate):
    tin = []
    for f2 in range(16):
        rr, ri, _ = yrows(16 * k1 + f2)
        tin.append((_ld(y_ref, qrow + rr), _ld(y_ref, qrow + ri)))
    Y = dft(tin, 1)
    for k2 in range(16):
        ifft_emit(s_ref, st_ref, srow, k1, k2, Y[k2], is_gate)


def ifft_passB1(y_ref, qrow, k1):
    locs = [yrows(16 * k1 + f2) for f2 in range(1, 16, 2)]
    O = dft([(_ld(y_ref, qrow + rr), _ld(y_ref, qrow + ri)) for rr, ri, _ in locs], 1)
    for k in range(8):
        t = cmulc(O[k], *croot(k, 16, 1))
        rr, ri, _ = locs[k]
        y_ref[pl.ds(qrow + rr, 8), :] = u32(vmat(t[0]))
        y_ref[pl.ds(qrow + ri, 8), :] = u32(vmat(t[1]))


def ifft_passB2(y_ref, s_ref, st_ref, srow, qrow, k1, is_gate):
    le = [yrows(16 * k1 + f2) for f2 in range(0, 16, 2)]
    lo = [yrows(16 * k1 + f2) for f2 in range(1, 16, 2)]
    E = dft([(_ld(y_ref, qrow + rr), _ld(y_ref, qrow + ri)) for rr, ri, _ in le], 1)
    for k in range(8):
        rr, ri, _ = lo[k]
        o = (_ld(y_ref, qrow + rr), _ld(y_ref, qrow + ri))
        if k1 + 8 * k >= KT - 1:
            ifft_emit(s_ref, st_ref, srow, k1, k, cadd(E[k], o), is_gate)
        ifft_emit(s_ref, st_ref, srow, k1, k + 8, csub(E[k], o), is_gate)


def ifft_pieces(y_ref, s_ref, st_ref, ob_ref, q, is_gate, ga, gb):
    qrow = pl.multiple_of(q * 16, 16)
    srow = pl.multiple_of(q * (16 * L), 16)
    pieces = []
    for f0 in range(0, 16, ga):
        def pa(f0=f0):
            for f2 in range(f0, f0 + ga):
                ifft_passA(y_ref, qrow, f2)
        pieces.append(pa)
    if gb == 0:
        for k1 in range(8):
            pieces.append(lambda k1=k1: ifft_passB1(y_ref, qrow, k1))
            pieces.append(lambda k1=k1: ifft_passB2(y_ref, s_ref, st_ref, srow, qrow, k1, is_gate))
        gb = 99
    for k0 in range(0, 8 if gb != 99 else 0, gb):
        def pb(k0=k0):
            for k1 in range(k0, k0 + gb):
                ifft_passB(y_ref, s_ref, st_ref, srow, qrow, k1, is_gate)
        pieces.append(pb)
    if is_gate:
        def cv():
            for i in range(L):
                ob_ref[pl.ds(srow + 16 * i, 16), :] = bf(st_ref[pl.ds(16 * i, 16), :])
        pieces.append(cv)
    return pieces


LANE0 = (0, 256, 128, 384)
RT = 16 * L
VB = 2 * BSTR


def make_kern(ga=1, gb=1, g1=1, g2=1, lead=2, w0n=4, xp=8, xahead=2, wtpace=True, tok=None, tailb=(0, 5, 11, 15, 18, 20, 21), upto=99):
  global TOKEN_ROWS
  if tok is not None:
    TOKEN_ROWS = tuple(tok)

  def kern(x_hbm, w_hbm, o_hbm, y0, y1, xh_ref, wh0, wh1, s_ref, st_ref, ws_ref, tw_ref, ob_ref, z_ref, xsem, wsem, osem, w0sem):
    ys = (y0, y1)
    whs = (wh0, wh1)
    xu = x_hbm.bitcast(jnp.uint32)
    wu = w_hbm.bitcast(jnp.uint32)

    XPIECE = 8000 // xp
    NXP = 2 * xp

    def xcp(p, h):
        b, i = divmod(p, xp)
        return pltpu.make_async_copy(xu.at[b, pl.ds(XPIECE * i, XPIECE), pl.ds(128 * h, 128)],
                                     ys[h].at[pl.ds(XOFF + b * BSTR + XPIECE * i, XPIECE)], xsem.at[2 * p + h])

    def wcp(c):
        return pltpu.make_async_copy(wu.at[:, :, pl.ds(LANE0[c], 128)], ws_ref.at[c % 2], wsem.at[c % 2])

    z_ref[0] = 0

    def w0cp(i):
        n = 128 // w0n
        return pltpu.make_async_copy(wu.at[:, pl.ds(n * i, n), pl.ds(LANE0[0], 128)], ws_ref.at[0, :, pl.ds(n * i, n), :], w0sem.at[i])
    for i in range(w0n):
        w0cp(i).start()
    XAHEAD = xahead
    for p in range(XAHEAD):
        for h in range(2):
            xcp(p, h).start()
    for h in range(2):
        ys[h][pl.ds(0, 32), :] = jnp.zeros((32, 128), jnp.uint32)
        ys[h][pl.ds(8032, 232), :] = jnp.zeros((232, 128), jnp.uint32)
        ys[h][pl.ds(16264, 232), :] = jnp.zeros((232, 128), jnp.uint32)

    def scale(c):
        return (0.5 if c % 2 == 1 else 1.0) / N

    def wt0_body(r, _):
        for i in range(w0n):
            @pl.when(r == i * (16 // w0n))
            def _():
                w0cp(i).wait()
        for p in wt_pieces(ws_ref.at[0], tw_ref, whs[0], r, scale(0)):
            p()
        return 0
    jax.lax.fori_loop(0, 16, wt0_body, 0)

    first_q = {}
    for p in range(NXP):
        b, i = divmod(p, xp)
        st = XOFF + b * BSTR + XPIECE * i
        first_q[p] = min(q for q in range(NQ) if 8 * L * q + 2 + 7 * L + N > st)

    def fwd_body(q, _):
        for p in range(NXP):
            @pl.when(q == first_q[p])
            def _():
                for h in range(2):
                    xcp(p, h).wait()
                if p + XAHEAD < NXP:
                    for h in range(2):
                        xcp(p + XAHEAD, h).start()
                if p == NXP - 1:
                    wcp(1).start()
                    wcp(2).start()
        fwd_column(ys, xh_ref, q)
        return 0
    jax.lax.fori_loop(0, NQ, fwd_body, 0)

    xh_u = xh_ref.bitcast(jnp.uint32)

    def ocp(hh, b, t0, n, k):
        return pltpu.make_async_copy(ob_ref.at[pl.ds(VB * b + t0, n)], o_hbm.at[b, pl.ds(t0, n), pl.ds(128 * hh, 128)], osem.at[k])

    def paced(pieces, tokens, ref, zero_row, lead, on=True):
        n = len(pieces)
        if not on:
            tokens = []
        for k, p in enumerate(pieces):
            if tokens and k >= lead:
                tk = tokens[((k - lead) * len(tokens)) // (n - lead + 1)]
                ref[pl.ds(zero_row, 8), :] = tk if ref.dtype == jnp.float32 else u32(tk)
            p()

    def phase(c_mm, c_if, c_wt, ranges):
        is_gate = c_if is not None and c_if % 2 == 1
        if c_mm is not None:
            wh_u = whs[c_mm % 2].bitcast(jnp.uint32)
            mm_special(xh_u, wh_u, ys[c_mm % 2])
        if c_wt is not None:
            wcp(c_wt).wait()

        def body(q, with_wt):
            tokens = []
            for s in range(3):
                tokens += mm_slot(xh_u, wh_u, ys[c_mm % 2], 3 * q + s)
            z = z_ref[0]
            if c_if is not None:
                yif = ys[c_if % 2]
                on = wtpace or not with_wt
                paced(ifft_pieces(yif, s_ref, st_ref, ob_ref, q, is_gate, ga, gb), tokens, yif,
                      pl.multiple_of(YROWS + z, 8), lead, on)
            if with_wt:
                paced(wt_pieces(ws_ref.at[c_wt % 2], tw_ref, whs[c_wt % 2], q, scale(c_wt), g1, g2), tokens, tw_ref,
                      pl.multiple_of(TWROWS + z, 8), lead, wtpace or c_if is None)

        for (q0, q1, after) in ranges:
            with_wt = c_wt is not None and q1 <= 16
            jax.lax.fori_loop(q0, q1, lambda q, _: (body(q, with_wt), 0)[1], 0)
            if after is not None:
                after()

    def nop():
        pass

    def out0_a():
        ocp(0, 0, 0, 16000, 0).start()
        ocp(0, 1, 0, 16 * RT - VB, 1).start()

    def out0_b():
        ocp(0, 1, 16 * RT - VB, 16000 - (16 * RT - VB), 2).start()

    def out0_wait():
        ocp(0, 0, 0, 16000, 0).wait()
        ocp(0, 1, 0, 16 * RT - VB, 1).wait()
        ocp(0, 1, 16 * RT - VB, 16000 - (16 * RT - VB), 2).wait()

    def out1_pieces():
        pcs = []
        for k in range(len(tailb) - 1):
            lo, hi = tailb[k] * RT, tailb[k + 1] * RT
            cur = []
            for b in range(2):
                a, e = max(lo, VB * b), min(hi, VB * b + 16000)
                if e > a:
                    cur.append((b, a - VB * b, e - a))
            pcs.append(cur)
        return pcs

    def out1(k, wait):
        for n, pc in enumerate(out1_pieces()[k]):
            cp = ocp(1, *pc, 3 + 2 * k + n)
            if wait:
                cp.wait()
            else:
                cp.start()

    def fin():
        z = z_ref[0]
        r = pl.ds(pl.multiple_of(z * 16, 16), 16)
        r8 = pl.ds(pl.multiple_of(z * 8, 8), 8)
        acc = xh_ref[z, z, z, r, :].astype(jnp.float32) + whs[0][z, z, r, :].astype(jnp.float32) + whs[1][z, z, r, :].astype(jnp.float32)
        acc = acc + s_ref[r, :].astype(jnp.float32) + ob_ref[r, :].astype(jnp.float32)
        acc = acc + jnp.concatenate([f32(ys[0][r8, :]), f32(ys[1][r8, :])], axis=0) + st_ref[r, :] + tw_ref[r, :]
        ob_ref[pl.ds(0, 16), :] = bf(acc)
        o = pltpu.make_async_copy(ob_ref.at[pl.ds(0, 16)], o_hbm.at[0, pl.ds(0, 16), pl.ds(0, 128)], osem.at[7])
        o.start(); o.wait()
    if upto == 0:
        wcp(1).wait(); wcp(2).wait(); fin(); return
    phase(0, None, 1, [(0, 16, None), (16, NQ, None)])
    if upto == 1:
        wcp(2).wait(); fin(); return
    wcp(3).start()
    phase(1, 0, 2, [(0, 16, None), (16, NQ, None)])
    if upto == 2:
        wcp(3).wait(); fin(); return
    phase(2, 1, 3, [(0, 16, out0_a), (16, NQ, out0_b)])
    if upto == 3:
        out0_wait(); fin(); return
    phase(3, 2, None, [(0, NQ, None)])
    out0_wait()
    if upto == 4:
        fin(); return

    def tail_body(q, _):
        for p in ifft_pieces(ys[1], s_ref, st_ref, ob_ref, q, True, 16, 8):
            p()
        return 0
    nseg = len(tailb) - 1

    def pick(i, vals):
        r = vals[-1]
        for k in range(len(vals) - 2, -1, -1):
            r = jnp.where(i == k, vals[k], r)
        return r

    def seg(i, _):
        jax.lax.fori_loop(pick(i, tailb[:-1]), pick(i, tailb[1:]), tail_body, 0)
        for k in range(nseg):
            @pl.when(i == k)
            def _():
                out1(k, False)
        return 0
    jax.lax.fori_loop(0, nseg, seg, 0)
    for k in range(nseg):
        out1(k, True)
  return kern


@jax.jit
def pallas_standalone__autoregressive_conv_wavernn__speech_kernel(x, w):
    kern = make_kern(**{"w0n": 2, "xp": 4})
    flags = None
    return pl.pallas_call(
        kern,
        in_specs=[pl.BlockSpec(memory_space=pl.ANY), pl.BlockSpec(memory_space=pl.ANY)],
        out_specs=pl.BlockSpec(memory_space=pl.ANY),
        out_shape=jax.ShapeDtypeStruct(x.shape, x.dtype),
        scratch_shapes=[
            pltpu.VMEM((YROWS + 8, 128), jnp.uint32), pltpu.VMEM((YROWS + 8, 128), jnp.uint32),
            pltpu.VMEM((NS, 3, 2, 336, 128), jnp.bfloat16),
            pltpu.VMEM((NS, 3, 256, 128), jnp.bfloat16),
            pltpu.VMEM((NS, 3, 256, 128), jnp.bfloat16),
            pltpu.VMEM((2 * VB, 128), jnp.bfloat16),
            pltpu.VMEM((RT, 128), jnp.float32),
            pltpu.VMEM((2, 31, 128, 128), jnp.uint32),
            pltpu.VMEM((TWROWS + 8, 128), jnp.float32),
            pltpu.VMEM((2 * VB, 128), jnp.bfloat16),
            pltpu.SMEM((1,), jnp.int32),
            pltpu.SemaphoreType.DMA((32,)), pltpu.SemaphoreType.DMA((2,)), pltpu.SemaphoreType.DMA((16,)), pltpu.SemaphoreType.DMA((8,)),
        ],
        compiler_params=pltpu.CompilerParams(vmem_limit_bytes=127 * 1024 * 1024, flags=flags),
    )(x, w)
```

```python
import math
import numpy as np
import jax
import jax.numpy as jnp
from jax.experimental import pallas as pl
from jax.experimental.pallas import tpu as pltpu

def vneg(a):
    return None if a is None else (a[0], -a[1])


def vadd(a, b):
    if a is None:
        return b
    if b is None:
        return a
    if a[1] > 0 and b[1] > 0:
        return (a[0] + b[0], 1)
    if a[1] > 0 and b[1] < 0:
        return (a[0] - b[0], 1)
    if a[1] < 0 and b[1] > 0:
        return (b[0] - a[0], 1)
    return (a[0] + b[0], -1)


def vsub(a, b):
    return vadd(a, vneg(b))


def vmulc(a, c):
    if a is None or c == 0.0:
        return None
    if c == 1.0:
        return a
    if c == -1.0:
        return vneg(a)
    return (a[0] * float(np.float32(c * a[1])), 1)


def vmat(a):
    return a[0] if a[1] > 0 else -a[0]


def cadd(a, b):
    return (vadd(a[0], b[0]), vadd(a[1], b[1]))


def csub(a, b):
    return (vsub(a[0], b[0]), vsub(a[1], b[1]))


def conj(a):
    return (a[0], vneg(a[1]))


def cmuli(a, s):
    return (vneg(a[1]), a[0]) if s > 0 else (a[1], vneg(a[0]))


def _snap(x):
    for v in (0.0, 1.0, -1.0):
        if abs(x - v) < 1e-12:
            return v
    return x


def croot(num, den, sgn):
    ang = sgn * 2.0 * math.pi * (num % den) / den
    return _snap(math.cos(ang)), _snap(math.sin(ang))


def cmulc(z, c, s):
    re, im = z
    if s == 0.0:
        return (vmulc(re, c), vmulc(im, c))
    if c == 0.0:
        return (vmulc(im, -s), vmulc(re, s))
    if im is None:
        return (vmulc(re, c), vmulc(re, s))
    if re is None:
        return (vmulc(im, -s), vmulc(im, c))
    if abs(abs(c) - abs(s)) < 1e-12:
        if s / c > 0:
            return (vmulc(vsub(re, im), c), vmulc(vadd(re, im), c))
        return (vmulc(vadd(re, im), c), vmulc(vsub(im, re), c))
    return (vsub(vmulc(re, c), vmulc(im, s)), vadd(vmulc(re, s), vmulc(im, c)))


def dft(xs, sgn):
    n = len(xs)
    if n == 1:
        return list(xs)
    if n == 2:
        return [cadd(xs[0], xs[1]), csub(xs[0], xs[1])]
    U = dft(xs[0::2], sgn)
    Z = dft(xs[1::4], sgn)
    Zp = dft(xs[3::4], sgn)
    out = [None] * n
    q = n // 4
    for k in range(q):
        t1 = cmulc(Z[k], *croot(k, n, sgn))
        t2 = cmulc(Zp[k], *croot(3 * k, n, sgn))
        s = cadd(t1, t2)
        d = cmuli(csub(t1, t2), sgn)
        out[k] = cadd(U[k], s)
        out[k + 2 * q] = csub(U[k], s)
        out[k + q] = cadd(U[k + q], d)
        out[k + 3 * q] = csub(U[k + q], d)
    return out


def rdft(xs):
    n = len(xs)
    if n == 1:
        return [(xs[0], None)]
    if n == 2:
        return [(vadd(xs[0], xs[1]), None), (vsub(xs[0], xs[1]), None)]
    E = rdft(xs[0::2])
    O = rdft(xs[1::2])
    out = [None] * (n // 2 + 1)
    for k in range(n // 4 + 1):
        t = cmulc(O[k], *croot(k, n, -1))
        out[k] = cadd(E[k], t)
        if k != n // 4:
            out[n // 2 - k] = conj(csub(E[k], t))
    return out


N = 128
KT = 31
L = N - KT + 1
NB = 84
NQ = 21
BSTR = NB * L
XOFF = 32
XROWS = 2 * BSTR + 32
TROWS = 9 * 8 * 2 * 16
XPIECE = 2000


def _slots():
    s = []
    for u in range(9):
        for k2 in range(8):
            if u == 0 and (k2 == 0 or k2 >= 4):
                continue
            if u == 8 and k2 > 3:
                continue
            s.append((u, k2))
    return s


SLOTS = _slots()
NG = len(SLOTS)
SP = NG
NS = NG + 1
SIDX = {uk: i for i, uk in enumerate(SLOTS)}
TOKEN_ROWS = (0, 40, 80, 120, 160)
YROWS = NS * 672
TWROWS = 9 * 8 * 2 * 16


def f32(u):
    return pltpu.bitcast(u, jnp.float32)


def u32(v):
    return pltpu.bitcast(v, jnp.uint32)


def bf(v):
    return v.astype(jnp.bfloat16)


def fwd_pass1(xs_ref, q, n2):
    base = 2 + q * (8 * L)
    xin = []
    for n1 in range(16):
        u = xs_ref[pl.ds(base + 8 * n1 + n2, 8, stride=L), :]
        xin.append(((f32(u << 16), 1), (f32(u & jnp.uint32(0xFFFF0000)), 1)))
    X1 = dft(xin, -1)
    for u in range(9):
        top = cmulc(X1[u], *croot(n2 * u, N, -1))
        kp = (16 - u) % 16
        bt = conj(cmulc(X1[kp], *croot(n2 * kp - (16 * n2 if u > 0 else 0), N, -1)))
        for ri in range(2):
            r0 = XROWS + ((u * 8 + n2) * 2 + ri) * 16
            xs_ref[pl.ds(r0, 8), :] = u32(vmat(top[ri]))
            xs_ref[pl.ds(r0 + 8, 8), :] = u32(vmat(bt[ri]))


def fwd_pass2(xs_ref, xh_ref, h, q, u):
    rows = pl.ds(pl.multiple_of(q * 16, 16), 16)
    zin = []
    for n2 in range(8):
        r0 = XROWS + ((u * 8 + n2) * 2) * 16
        zin.append(((f32(xs_ref[pl.ds(r0, 16), :]), 1), (f32(xs_ref[pl.ds(r0 + 16, 16), :]), 1)))
    X2 = dft(zin, -1)
    for k2 in range(8):
        if u == 0 and k2 in (0, 4):
            a, b = vmat(X2[k2][0]), vmat(X2[k2][1])
            xh_ref[SP, k2 // 4, h, rows, :] = bf(jnp.concatenate([a[0:8], b[0:8]], axis=0))
        if (u, k2) not in SIDX:
            continue
        j = SIDX[u, k2]
        a, b = X2[k2]
        xh_ref[j, 0, h, rows, :] = bf(vmat(a))
        xh_ref[j, 1, h, rows, :] = bf(vmat(b))
        xh_ref[j, 2, h, rows, :] = bf(vmat(vadd(a, b)))


def fwd_column(xs, xh_ref, q):
    for n2 in range(8):
        for h in range(2):
            fwd_pass1(xs[h], q, n2)
    for u in range(9):
        for h in range(2):
            fwd_pass2(xs[h], xh_ref, h, q, u)


def _wt_nonzero():
    class _P:
        def __add__(self, o): return self
        __sub__ = __mul__ = __radd__ = __rsub__ = __rmul__ = __add__
    nz = {}
    for rr in range(8):
        Y = rdft([(_P(), 1) if rr + 8 * m < KT else None for m in range(16)])
        for u in range(9):
            t = cmulc(Y[u], *croot(rr * u, N, -1))
            for ri in range(2):
                nz[rr, u, ri] = t[ri] is not None
    return nz


WT_NONZERO = _wt_nonzero()


def wt_pieces(ws, tw_ref, wh_ref, r, scale, g1=2, g2=2):
    r8 = pl.ds(pl.multiple_of(r * 8, 8), 8)
    rows = pl.ds(pl.multiple_of(r * 16, 16), 16)

    def tap(j):
        if j >= KT:
            return None
        wv = pltpu.bitcast(ws[KT - 1 - j, r8, :], jnp.bfloat16)
        return (wv.astype(jnp.float32) * float(scale), 1)

    def p1(rr):
        Y = rdft([tap(rr + 8 * m) for m in range(16)])
        for u in range(9):
            t = cmulc(Y[u], *croot(rr * u, N, -1))
            for ri in range(2):
                if t[ri] is not None:
                    tw_ref[pl.ds(((u * 8 + rr) * 2 + ri) * 16, 16), :] = vmat(t[ri])

    def p2(u):
        def ld(rr, ri):
            if not WT_NONZERO[rr, u, ri]:
                return None
            return (tw_ref[pl.ds(((u * 8 + rr) * 2 + ri) * 16, 16), :], 1)
        if u == 0:
            X2 = rdft([ld(rr, 0) for rr in range(8)])
        else:
            X2 = dft([(ld(rr, 0), ld(rr, 1)) for rr in range(8)], -1)
        for k2 in range(8):
            if u == 0 and k2 in (0, 4):
                wh_ref[SP, k2 // 4, rows, :] = bf(vmat(X2[k2][0]))
            if (u, k2) not in SIDX:
                continue
            j = SIDX[u, k2]
            c, d = X2[k2]
            wh_ref[j, 0, rows, :] = bf(vmat(c))
            wh_ref[j, 1, rows, :] = bf(vmat(vsub(d, c)))
            wh_ref[j, 2, rows, :] = bf(vmat(vadd(c, d)))

    pieces = []
    for r0 in range(0, 8, g1):
        pieces.append(lambda r0=r0: [p1(rr) for rr in range(r0, r0 + g1)])
    us = [1, 2, 3, 4, 5, 6, 7, 0, 8]
    for i in range(0, 9, g2):
        pieces.append(lambda i=i: [p2(u) for u in us[i:i + g2]])
    return pieces


def _lhs(xh_u, j, t):
    return jnp.concatenate([pltpu.bitcast(xh_u[j, t, h], jnp.bfloat16) for h in range(2)], axis=1)


def _rhs(wh_u, j, t):
    return pltpu.bitcast(wh_u[j, t], jnp.bfloat16)


def _dot(a, b):
    return jnp.dot(a, b, preferred_element_type=jnp.float32)


def mm_slot(xh_u, wh_u, y_ref, j):
    base = pl.multiple_of(j * 672, 16) if not isinstance(j, int) else j * 672
    rre, rim = pl.ds(base, 336), pl.ds(base + 336, 336)
    k1 = _dot(_lhs(xh_u, j, 2), _rhs(wh_u, j, 0))
    y_ref[rre, :] = u32(k1)
    k2 = _dot(_lhs(xh_u, j, 0), _rhs(wh_u, j, 1))
    y_ref[rim, :] = u32(f32(y_ref[rre, :]) + k2)
    k3 = _dot(_lhs(xh_u, j, 1), _rhs(wh_u, j, 2))
    y_ref[rre, :] = u32(f32(y_ref[rre, :]) - k3)
    return [k[r:r + 8] for k in (k1, k2, k3) for r in TOKEN_ROWS]


def mm_special(xh_u, wh_u, y_ref):
    for t in range(2):
        y_ref[pl.ds(SP * 672 + 336 * t, 336), :] = u32(_dot(_lhs(xh_u, SP, t), _rhs(wh_u, SP, t)))


def yrows(f):
    f2, f1 = f % 16, f // 16
    if f == 0:
        return SP * 672, SP * 672 + 8, 1
    if f == 64:
        return SP * 672 + 336, SP * 672 + 344, 1
    if 1 <= f2 <= 7:
        j, tb = SIDX[f2, f1], 0
    elif f2 >= 9:
        j, tb = SIDX[16 - f2, 7 - f1], 1
    elif f2 == 0:
        j, tb = (SIDX[0, f1], 0) if f1 < 4 else (SIDX[0, 8 - f1], 1)
    else:
        j, tb = (SIDX[8, f1], 0) if f1 <= 3 else (SIDX[8, 7 - f1], 1)
    r = j * 672 + 8 * tb
    return r, r + 336, (-1 if tb else 1)


def ifft_passA(y_ref, qrow, f2):
    locs = [yrows(16 * f1 + f2) for f1 in range(8)]
    yin = []
    for (rr, ri, sg) in locs:
        yin.append(((f32(y_ref[pl.ds(qrow + rr, 8), :]), 1), (f32(y_ref[pl.ds(qrow + ri, 8), :]), sg)))
    A = dft(yin, 1)
    for k1 in range(8):
        t = cmulc(A[k1], *croot(f2 * k1, N, 1))
        rr, ri, _ = locs[k1]
        y_ref[pl.ds(qrow + rr, 8), :] = u32(vmat(t[0]))
        y_ref[pl.ds(qrow + ri, 8), :] = u32(vmat(t[1]))


def _ld(y_ref, r):
    return (f32(y_ref[pl.ds(r, 8), :]), 1)


def ifft_emit(s_ref, st_ref, srow, k1, k2, y, is_gate):
    n = k1 + 8 * k2
    if n < KT - 1:
        return
    m = n - (KT - 1)
    for part in range(2):
        v = jnp.tanh(vmat(y[part]))
        idx = pl.ds(srow + (2 * m + part), 8, stride=2 * L)
        if is_gate:
            v = s_ref[idx, :] * (0.5 * v + 0.5)
        s_ref[idx, :] = v


def ifft_passB(y_ref, s_ref, st_ref, srow, qrow, k1, is_gate):
    tin = []
    for f2 in range(16):
        rr, ri, _ = yrows(16 * k1 + f2)
        tin.append((_ld(y_ref, qrow + rr), _ld(y_ref, qrow + ri)))
    Y = dft(tin, 1)
    for k2 in range(16):
        ifft_emit(s_ref, st_ref, srow, k1, k2, Y[k2], is_gate)


def ifft_passB1(y_ref, qrow, k1):
    locs = [yrows(16 * k1 + f2) for f2 in range(1, 16, 2)]
    O = dft([(_ld(y_ref, qrow + rr), _ld(y_ref, qrow + ri)) for rr, ri, _ in locs], 1)
    for k in range(8):
        t = cmulc(O[k], *croot(k, 16, 1))
        rr, ri, _ = locs[k]
        y_ref[pl.ds(qrow + rr, 8), :] = u32(vmat(t[0]))
        y_ref[pl.ds(qrow + ri, 8), :] = u32(vmat(t[1]))


def ifft_passB2(y_ref, s_ref, st_ref, srow, qrow, k1, is_gate):
    le = [yrows(16 * k1 + f2) for f2 in range(0, 16, 2)]
    lo = [yrows(16 * k1 + f2) for f2 in range(1, 16, 2)]
    E = dft([(_ld(y_ref, qrow + rr), _ld(y_ref, qrow + ri)) for rr, ri, _ in le], 1)
    for k in range(8):
        rr, ri, _ = lo[k]
        o = (_ld(y_ref, qrow + rr), _ld(y_ref, qrow + ri))
        if k1 + 8 * k >= KT - 1:
            ifft_emit(s_ref, st_ref, srow, k1, k, cadd(E[k], o), is_gate)
        ifft_emit(s_ref, st_ref, srow, k1, k + 8, csub(E[k], o), is_gate)


def convert(s_ref, ob_ref, q):
    srow = pl.multiple_of(q * (16 * L), 16) if not isinstance(q, int) else q * 16 * L
    obv = ob_ref.at[pl.ds(srow, 16 * L)]
    for i in range(L):
        obv[pl.ds(16 * i, 16), :] = bf(s_ref[pl.ds(srow + 16 * i, 16), :])


def ifft_pieces(y_ref, s_ref, st_ref, ob_ref, q, is_gate, ga, gb, lagcv=False):
    qrow = pl.multiple_of(q * 16, 16)
    srow = pl.multiple_of(q * (16 * L), 16)
    pieces = []
    for f0 in range(0, 16, ga):
        def pa(f0=f0):
            for f2 in range(f0, f0 + ga):
                ifft_passA(y_ref, qrow, f2)
        pieces.append(pa)
    if gb == 0:
        for k1 in range(8):
            pieces.append(lambda k1=k1: ifft_passB1(y_ref, qrow, k1))
            pieces.append(lambda k1=k1: ifft_passB2(y_ref, s_ref, st_ref, srow, qrow, k1, is_gate))
        gb = 99
    for k0 in range(0, 8 if gb != 99 else 0, gb):
        def pb(k0=k0):
            for k1 in range(k0, k0 + gb):
                ifft_passB(y_ref, s_ref, st_ref, srow, qrow, k1, is_gate)
        pieces.append(pb)
    if is_gate and not lagcv:
        pieces.append(lambda: convert(s_ref, ob_ref, q))
    return pieces


LANE0 = (0, 256, 128, 384)
RT = 16 * L
VB = 2 * BSTR


def make_kern(ga=1, gb=1, g1=1, g2=1, lead=2, w0n=4, xp=8, xahead=2, wtpace=True, lagcv=True, wi=None, ww=None, tok=None, tailb=(0, 5, 11, 15, 18, 20, 21), upto=99):
  global TOKEN_ROWS
  if tok is not None:
    TOKEN_ROWS = tuple(tok)

  def kern(x_hbm, w_hbm, o_hbm, y0, y1, xh_ref, wh0, wh1, s_ref, st_ref, ws_ref, tw_ref, ob_ref, z_ref, xsem, wsem, osem, w0sem):
    ys = (y0, y1)
    whs = (wh0, wh1)
    xu = x_hbm.bitcast(jnp.uint32)
    wu = w_hbm.bitcast(jnp.uint32)

    XPIECE = 8000 // xp
    NXP = 2 * xp

    def xcp(p, h):
        b, i = divmod(p, xp)
        return pltpu.make_async_copy(xu.at[b, pl.ds(XPIECE * i, XPIECE), pl.ds(128 * h, 128)],
                                     ys[h].at[pl.ds(XOFF + b * BSTR + XPIECE * i, XPIECE)], xsem.at[2 * p + h])

    def wcp(c):
        return pltpu.make_async_copy(wu.at[:, :, pl.ds(LANE0[c], 128)], ws_ref.at[0], wsem.at[0])

    z_ref[0] = 0

    def w0cp(i):
        n = 128 // w0n
        return pltpu.make_async_copy(wu.at[:, pl.ds(n * i, n), pl.ds(LANE0[0], 128)], ws_ref.at[0, :, pl.ds(n * i, n), :], w0sem.at[i])
    for i in range(w0n):
        w0cp(i).start()
    XAHEAD = xahead
    for p in range(XAHEAD):
        for h in range(2):
            xcp(p, h).start()
    for h in range(2):
        ys[h][pl.ds(0, 32), :] = jnp.zeros((32, 128), jnp.uint32)
        ys[h][pl.ds(8032, 232), :] = jnp.zeros((232, 128), jnp.uint32)
        ys[h][pl.ds(16264, 232), :] = jnp.zeros((232, 128), jnp.uint32)

    def scale(c):
        return (0.5 if c % 2 == 1 else 1.0) / N

    def wt0_body(r, _):
        for i in range(w0n):
            @pl.when(r == i * (16 // w0n))
            def _():
                w0cp(i).wait()
        for p in wt_pieces(ws_ref.at[0], tw_ref, whs[0], r, scale(0)):
            p()
        return 0
    jax.lax.fori_loop(0, 16, wt0_body, 0)

    first_q = {}
    for p in range(NXP):
        b, i = divmod(p, xp)
        st = XOFF + b * BSTR + XPIECE * i
        first_q[p] = min(q for q in range(NQ) if 8 * L * q + 2 + 7 * L + N > st)

    def fwd_body(q, _):
        for p in range(NXP):
            @pl.when(q == first_q[p])
            def _():
                for h in range(2):
                    xcp(p, h).wait()
                if p + XAHEAD < NXP:
                    for h in range(2):
                        xcp(p + XAHEAD, h).start()
                if p == NXP - 1:
                    wcp(1).start()
        fwd_column(ys, xh_ref, q)
        return 0
    jax.lax.fori_loop(0, NQ, fwd_body, 0)

    xh_u = xh_ref.bitcast(jnp.uint32)

    def ocp(hh, b, t0, n, k):
        return pltpu.make_async_copy(ob_ref.at[pl.ds(VB * b + t0, n)], o_hbm.at[b, pl.ds(t0, n), pl.ds(128 * hh, 128)], osem.at[k])

    def paced_w(pieces, weights, tokens, ref, zero_row, lead, span, off):
        tot = float(sum(weights[lead:]))
        cum = 0.0
        for k, p in enumerate(pieces):
            if k >= lead:
                idx = int(off + cum / tot * span * len(tokens))
                tk = tokens[max(0, min(idx, len(tokens) - 1))]
                ref[pl.ds(zero_row, 8), :] = tk if ref.dtype == jnp.float32 else u32(tk)
                cum += weights[k]
            else:
                pass
            p()

    def paced(pieces, tokens, ref, zero_row, lead, on=True):
        n = len(pieces)
        if not on:
            tokens = []
        for k, p in enumerate(pieces):
            if tokens and k >= lead:
                tk = tokens[((k - lead) * len(tokens)) // (n - lead + 1)]
                ref[pl.ds(zero_row, 8), :] = tk if ref.dtype == jnp.float32 else u32(tk)
            p()

    def phase(c_mm, c_if, c_wt, ranges):
        is_gate = c_if is not None and c_if % 2 == 1
        if c_mm is not None:
            wh_u = whs[c_mm % 2].bitcast(jnp.uint32)
            mm_special(xh_u, wh_u, ys[c_mm % 2])
        if c_wt is not None:
            wcp(c_wt).wait()

        def body(q, with_wt):
            tokens = []
            for s in range(3):
                tokens += mm_slot(xh_u, wh_u, ys[c_mm % 2], 3 * q + s)
            z = z_ref[0]
            if is_gate and lagcv:
                convert(s_ref, ob_ref, jnp.maximum(q - 1, 0))
            if c_if is not None:
                yif = ys[c_if % 2]
                on = wtpace or not with_wt
                if wi is not None:
                    pcs = ifft_pieces(yif, s_ref, st_ref, ob_ref, q, is_gate, ga, gb, lagcv)
                    wa, wb, span, off, ld = wi
                    paced_w(pcs, [wa] * 16 + [wb] * (len(pcs) - 16), tokens, yif, pl.multiple_of(YROWS + z, 8), ld, span, off)
                else:
                    paced(ifft_pieces(yif, s_ref, st_ref, ob_ref, q, is_gate, ga, gb, lagcv), tokens, yif,
                          pl.multiple_of(YROWS + z, 8), lead, on)
            if with_wt and ww is not None:
                pcs = wt_pieces(ws_ref.at[0], tw_ref, whs[c_wt % 2], q, scale(c_wt), g1, g2)
                w1, w2, span, off, ld = ww
                n1 = 8 // g1
                paced_w(pcs, [w1] * n1 + [w2] * (len(pcs) - n1), tokens, tw_ref, pl.multiple_of(TWROWS + z, 8), ld, span, off)
            elif with_wt:
                paced(wt_pieces(ws_ref.at[0], tw_ref, whs[c_wt % 2], q, scale(c_wt), g1, g2), tokens, tw_ref,
                      pl.multiple_of(TWROWS + z, 8), lead, wtpace or c_if is None)

        for (q0, q1, after) in ranges:
            with_wt = c_wt is not None and q1 <= 16
            jax.lax.fori_loop(q0, q1, lambda q, _: (body(q, with_wt), 0)[1], 0)
            if after is not None:
                after()

    def nop():
        pass

    NA = 15 if lagcv else 16

    def out0_a():
        ocp(0, 0, 0, 16000, 0).start()
        ocp(0, 1, 0, NA * RT - VB, 1).start()

    def out0_b():
        if lagcv:
            convert(s_ref, ob_ref, NQ - 1)
        ocp(0, 1, NA * RT - VB, 16000 - (NA * RT - VB), 2).start()

    def out0_wait():
        ocp(0, 0, 0, 16000, 0).wait()
        ocp(0, 1, 0, NA * RT - VB, 1).wait()
        ocp(0, 1, NA * RT - VB, 16000 - (NA * RT - VB), 2).wait()

    def out1_pieces():
        pcs = []
        for k in range(len(tailb) - 1):
            lo, hi = tailb[k] * RT, tailb[k + 1] * RT
            cur = []
            for b in range(2):
                a, e = max(lo, VB * b), min(hi, VB * b + 16000)
                if e > a:
                    cur.append((b, a - VB * b, e - a))
            pcs.append(cur)
        return pcs

    def out1(k, wait):
        for n, pc in enumerate(out1_pieces()[k]):
            cp = ocp(1, *pc, 3 + 2 * k + n)
            if wait:
                cp.wait()
            else:
                cp.start()

    def fin():
        z = z_ref[0]
        r = pl.ds(pl.multiple_of(z * 16, 16), 16)
        r8 = pl.ds(pl.multiple_of(z * 8, 8), 8)
        acc = xh_ref[z, z, z, r, :].astype(jnp.float32) + whs[0][z, z, r, :].astype(jnp.float32) + whs[1][z, z, r, :].astype(jnp.float32)
        acc = acc + s_ref[r, :] + ob_ref[r, :].astype(jnp.float32)
        acc = acc + jnp.concatenate([f32(ys[0][r8, :]), f32(ys[1][r8, :])], axis=0) + tw_ref[r, :]
        ob_ref[pl.ds(0, 16), :] = bf(acc)
        o = pltpu.make_async_copy(ob_ref.at[pl.ds(0, 16)], o_hbm.at[0, pl.ds(0, 16), pl.ds(0, 128)], osem.at[7])
        o.start(); o.wait()
    if upto == 0:
        wcp(1).wait(); fin(); return
    phase(0, None, 1, [(0, 16, lambda: wcp(2).start()), (16, NQ, None)])
    if upto == 1:
        wcp(2).wait(); fin(); return
    phase(1, 0, 2, [(0, 16, lambda: wcp(3).start()), (16, NQ, None)])
    if upto == 2:
        wcp(3).wait(); fin(); return
    phase(2, 1, 3, [(0, 16, out0_a), (16, NQ, out0_b)])
    if upto == 3:
        out0_wait(); fin(); return
    phase(3, 2, None, [(0, NQ, None)])
    out0_wait()
    if upto == 4:
        fin(); return

    def tail_body(q, _):
        if lagcv:
            convert(s_ref, ob_ref, jnp.maximum(q - 1, 0))
        for p in ifft_pieces(ys[1], s_ref, st_ref, ob_ref, q, True, 16, 8, lagcv):
            p()
        return 0
    nseg = len(tailb) - 1

    def pick(i, vals):
        r = vals[-1]
        for k in range(len(vals) - 2, -1, -1):
            r = jnp.where(i == k, vals[k], r)
        return r

    def seg(i, _):
        if lagcv:
            lb = [0] + [min(b + 1, NQ) for b in tailb[1:]]
            jax.lax.fori_loop(pick(i, lb[:-1]), pick(i, lb[1:]), tail_body, 0)

            @pl.when(i == nseg - 1)
            def _():
                convert(s_ref, ob_ref, NQ - 1)
        else:
            jax.lax.fori_loop(pick(i, tailb[:-1]), pick(i, tailb[1:]), tail_body, 0)
        for k in range(nseg):
            @pl.when(i == k)
            def _():
                out1(k, False)
        return 0
    jax.lax.fori_loop(0, nseg, seg, 0)
    for k in range(nseg):
        out1(k, True)
  return kern


@jax.jit
def pallas_standalone__autoregressive_conv_wavernn__speech_kernel(x, w):
    kern = make_kern(**{"w0n": 2, "xp": 4, "g1": 2, "g2": 2})
    flags = None
    return pl.pallas_call(
        kern,
        in_specs=[pl.BlockSpec(memory_space=pl.ANY), pl.BlockSpec(memory_space=pl.ANY)],
        out_specs=pl.BlockSpec(memory_space=pl.ANY),
        out_shape=jax.ShapeDtypeStruct(x.shape, x.dtype),
        scratch_shapes=[
            pltpu.VMEM((YROWS + 8, 128), jnp.uint32), pltpu.VMEM((YROWS + 8, 128), jnp.uint32),
            pltpu.VMEM((NS, 3, 2, 336, 128), jnp.bfloat16),
            pltpu.VMEM((NS, 3, 256, 128), jnp.bfloat16),
            pltpu.VMEM((NS, 3, 256, 128), jnp.bfloat16),
            pltpu.VMEM((2 * VB, 128), jnp.float32),
            pltpu.VMEM((8, 128), jnp.float32),
            pltpu.VMEM((1, 31, 128, 128), jnp.uint32),
            pltpu.VMEM((TWROWS + 8, 128), jnp.float32),
            pltpu.VMEM((2 * VB, 128), jnp.bfloat16),
            pltpu.SMEM((1,), jnp.int32),
            pltpu.SemaphoreType.DMA((32,)), pltpu.SemaphoreType.DMA((2,)), pltpu.SemaphoreType.DMA((16,)), pltpu.SemaphoreType.DMA((8,)),
        ],
        compiler_params=pltpu.CompilerParams(vmem_limit_bytes=127 * 1024 * 1024, flags=flags),
    )(x, w)
```

```python
import math
import numpy as np
import jax
import jax.numpy as jnp
from jax.experimental import pallas as pl
from jax.experimental.pallas import tpu as pltpu

def vneg(a):
    return None if a is None else (a[0], -a[1])


def vadd(a, b):
    if a is None:
        return b
    if b is None:
        return a
    if a[1] > 0 and b[1] > 0:
        return (a[0] + b[0], 1)
    if a[1] > 0 and b[1] < 0:
        return (a[0] - b[0], 1)
    if a[1] < 0 and b[1] > 0:
        return (b[0] - a[0], 1)
    return (a[0] + b[0], -1)


def vsub(a, b):
    return vadd(a, vneg(b))


def vmulc(a, c):
    if a is None or c == 0.0:
        return None
    if c == 1.0:
        return a
    if c == -1.0:
        return vneg(a)
    return (a[0] * float(np.float32(c * a[1])), 1)


def vmat(a):
    return a[0] if a[1] > 0 else -a[0]


def cadd(a, b):
    return (vadd(a[0], b[0]), vadd(a[1], b[1]))


def csub(a, b):
    return (vsub(a[0], b[0]), vsub(a[1], b[1]))


def conj(a):
    return (a[0], vneg(a[1]))


def cmuli(a, s):
    return (vneg(a[1]), a[0]) if s > 0 else (a[1], vneg(a[0]))


def _snap(x):
    for v in (0.0, 1.0, -1.0):
        if abs(x - v) < 1e-12:
            return v
    return x


def croot(num, den, sgn):
    ang = sgn * 2.0 * math.pi * (num % den) / den
    return _snap(math.cos(ang)), _snap(math.sin(ang))


def cmulc(z, c, s):
    re, im = z
    if s == 0.0:
        return (vmulc(re, c), vmulc(im, c))
    if c == 0.0:
        return (vmulc(im, -s), vmulc(re, s))
    if im is None:
        return (vmulc(re, c), vmulc(re, s))
    if re is None:
        return (vmulc(im, -s), vmulc(im, c))
    if abs(abs(c) - abs(s)) < 1e-12:
        if s / c > 0:
            return (vmulc(vsub(re, im), c), vmulc(vadd(re, im), c))
        return (vmulc(vadd(re, im), c), vmulc(vsub(im, re), c))
    return (vsub(vmulc(re, c), vmulc(im, s)), vadd(vmulc(re, s), vmulc(im, c)))


def dft(xs, sgn):
    n = len(xs)
    if n == 1:
        return list(xs)
    if n == 2:
        return [cadd(xs[0], xs[1]), csub(xs[0], xs[1])]
    U = dft(xs[0::2], sgn)
    Z = dft(xs[1::4], sgn)
    Zp = dft(xs[3::4], sgn)
    out = [None] * n
    q = n // 4
    for k in range(q):
        t1 = cmulc(Z[k], *croot(k, n, sgn))
        t2 = cmulc(Zp[k], *croot(3 * k, n, sgn))
        s = cadd(t1, t2)
        d = cmuli(csub(t1, t2), sgn)
        out[k] = cadd(U[k], s)
        out[k + 2 * q] = csub(U[k], s)
        out[k + q] = cadd(U[k + q], d)
        out[k + 3 * q] = csub(U[k + q], d)
    return out


def rdft(xs):
    n = len(xs)
    if n == 1:
        return [(xs[0], None)]
    if n == 2:
        return [(vadd(xs[0], xs[1]), None), (vsub(xs[0], xs[1]), None)]
    E = rdft(xs[0::2])
    O = rdft(xs[1::2])
    out = [None] * (n // 2 + 1)
    for k in range(n // 4 + 1):
        t = cmulc(O[k], *croot(k, n, -1))
        out[k] = cadd(E[k], t)
        if k != n // 4:
            out[n // 2 - k] = conj(csub(E[k], t))
    return out


N = 128
KT = 31
L = N - KT + 1
NB = 84
NQ = 21
BSTR = NB * L
XOFF = 32
XROWS = 2 * BSTR + 32
TROWS = 9 * 8 * 2 * 16
XPIECE = 2000


def _slots():
    s = []
    for u in range(9):
        for k2 in range(8):
            if u == 0 and (k2 == 0 or k2 >= 4):
                continue
            if u == 8 and k2 > 3:
                continue
            s.append((u, k2))
    return s


SLOTS = _slots()
NG = len(SLOTS)
SP = NG
NS = NG + 1
SIDX = {uk: i for i, uk in enumerate(SLOTS)}
YROWS = NS * 672
TWROWS = 9 * 8 * 2 * 16


def f32(u):
    return pltpu.bitcast(u, jnp.float32)


def u32(v):
    return pltpu.bitcast(v, jnp.uint32)


def bf(v):
    return v.astype(jnp.bfloat16)


def fwd_pass1(xs_ref, q, n2):
    base = 2 + q * (8 * L)
    xin = []
    for n1 in range(16):
        u = xs_ref[pl.ds(base + 8 * n1 + n2, 8, stride=L), :]
        xin.append(((f32(u << 16), 1), (f32(u & jnp.uint32(0xFFFF0000)), 1)))
    X1 = dft(xin, -1)
    for u in range(9):
        top = cmulc(X1[u], *croot(n2 * u, N, -1))
        kp = (16 - u) % 16
        bt = conj(cmulc(X1[kp], *croot(n2 * kp - (16 * n2 if u > 0 else 0), N, -1)))
        for ri in range(2):
            r0 = XROWS + ((u * 8 + n2) * 2 + ri) * 16
            xs_ref[pl.ds(r0, 8), :] = u32(vmat(top[ri]))
            xs_ref[pl.ds(r0 + 8, 8), :] = u32(vmat(bt[ri]))


def fwd_pass2(xs_ref, xh_ref, h, q, u):
    rows = pl.ds(pl.multiple_of(q * 16, 16), 16)
    zin = []
    for n2 in range(8):
        r0 = XROWS + ((u * 8 + n2) * 2) * 16
        zin.append(((f32(xs_ref[pl.ds(r0, 16), :]), 1), (f32(xs_ref[pl.ds(r0 + 16, 16), :]), 1)))
    X2 = dft(zin, -1)
    for k2 in range(8):
        if u == 0 and k2 in (0, 4):
            a, b = vmat(X2[k2][0]), vmat(X2[k2][1])
            xh_ref[SP, k2 // 4, h, rows, :] = bf(jnp.concatenate([a[0:8], b[0:8]], axis=0))
        if (u, k2) not in SIDX:
            continue
        j = SIDX[u, k2]
        a, b = X2[k2]
        xh_ref[j, 0, h, rows, :] = bf(vmat(a))
        xh_ref[j, 1, h, rows, :] = bf(vmat(b))
        xh_ref[j, 2, h, rows, :] = bf(vmat(vadd(a, b)))


def fwd_column(xs, xh_ref, q):
    for n2 in range(8):
        for h in range(2):
            fwd_pass1(xs[h], q, n2)
    for u in range(9):
        for h in range(2):
            fwd_pass2(xs[h], xh_ref, h, q, u)


def _wt_nonzero():
    class _P:
        def __add__(self, o): return self
        __sub__ = __mul__ = __radd__ = __rsub__ = __rmul__ = __add__
    nz = {}
    for rr in range(8):
        Y = rdft([(_P(), 1) if rr + 8 * m < KT else None for m in range(16)])
        for u in range(9):
            t = cmulc(Y[u], *croot(rr * u, N, -1))
            for ri in range(2):
                nz[rr, u, ri] = t[ri] is not None
    return nz


WT_NONZERO = _wt_nonzero()


def wt_pieces(ws, tw_ref, wh_ref, r, scale, g1=2, g2=2):
    r8 = pl.ds(pl.multiple_of(r * 8, 8), 8)
    rows = pl.ds(pl.multiple_of(r * 16, 16), 16)

    def tap(j):
        if j >= KT:
            return None
        wv = pltpu.bitcast(ws[KT - 1 - j, r8, :], jnp.bfloat16)
        return (wv.astype(jnp.float32) * float(scale), 1)

    def p1(rr):
        Y = rdft([tap(rr + 8 * m) for m in range(16)])
        for u in range(9):
            t = cmulc(Y[u], *croot(rr * u, N, -1))
            for ri in range(2):
                if t[ri] is not None:
                    tw_ref[pl.ds(((u * 8 + rr) * 2 + ri) * 16, 16), :] = vmat(t[ri])

    def p2(u):
        def ld(rr, ri):
            if not WT_NONZERO[rr, u, ri]:
                return None
            return (tw_ref[pl.ds(((u * 8 + rr) * 2 + ri) * 16, 16), :], 1)
        if u == 0:
            X2 = rdft([ld(rr, 0) for rr in range(8)])
        else:
            X2 = dft([(ld(rr, 0), ld(rr, 1)) for rr in range(8)], -1)
        for k2 in range(8):
            if u == 0 and k2 in (0, 4):
                wh_ref[SP, k2 // 4, rows, :] = bf(vmat(X2[k2][0]))
            if (u, k2) not in SIDX:
                continue
            j = SIDX[u, k2]
            c, d = X2[k2]
            wh_ref[j, 0, rows, :] = bf(vmat(c))
            wh_ref[j, 1, rows, :] = bf(vmat(vsub(d, c)))
            wh_ref[j, 2, rows, :] = bf(vmat(vadd(c, d)))

    pieces = []
    for r0 in range(0, 8, g1):
        pieces.append(lambda r0=r0: [p1(rr) for rr in range(r0, r0 + g1)])
    us = [1, 2, 3, 4, 5, 6, 7, 0, 8]
    for i in range(0, 9, g2):
        pieces.append(lambda i=i: [p2(u) for u in us[i:i + g2]])
    return pieces


def _lhs(xh_u, j, t):
    return jnp.concatenate([pltpu.bitcast(xh_u[j, t, h], jnp.bfloat16) for h in range(2)], axis=1)


def _rhs(wh_u, j, t):
    return pltpu.bitcast(wh_u[j, t], jnp.bfloat16)


def _dot(a, b):
    return jnp.dot(a, b, preferred_element_type=jnp.float32)


def mm_slot(xh_u, wh_u, y_ref, j, token_rows):
    base = pl.multiple_of(j * 672, 16) if not isinstance(j, int) else j * 672
    rre, rim = pl.ds(base, 336), pl.ds(base + 336, 336)
    k1 = _dot(_lhs(xh_u, j, 2), _rhs(wh_u, j, 0))
    y_ref[rre, :] = u32(k1)
    k2 = _dot(_lhs(xh_u, j, 0), _rhs(wh_u, j, 1))
    y_ref[rim, :] = u32(f32(y_ref[rre, :]) + k2)
    k3 = _dot(_lhs(xh_u, j, 1), _rhs(wh_u, j, 2))
    y_ref[rre, :] = u32(f32(y_ref[rre, :]) - k3)
    return [k[r:r + 8] for k in (k1, k2, k3) for r in token_rows]


def mm_special(xh_u, wh_u, y_ref):
    for t in range(2):
        y_ref[pl.ds(SP * 672 + 336 * t, 336), :] = u32(_dot(_lhs(xh_u, SP, t), _rhs(wh_u, SP, t)))


def yrows(f):
    f2, f1 = f % 16, f // 16
    if f == 0:
        return SP * 672, SP * 672 + 8, 1
    if f == 64:
        return SP * 672 + 336, SP * 672 + 344, 1
    if 1 <= f2 <= 7:
        j, tb = SIDX[f2, f1], 0
    elif f2 >= 9:
        j, tb = SIDX[16 - f2, 7 - f1], 1
    elif f2 == 0:
        j, tb = (SIDX[0, f1], 0) if f1 < 4 else (SIDX[0, 8 - f1], 1)
    else:
        j, tb = (SIDX[8, f1], 0) if f1 <= 3 else (SIDX[8, 7 - f1], 1)
    r = j * 672 + 8 * tb
    return r, r + 336, (-1 if tb else 1)


def ifft_passA(y_ref, qrow, f2):
    locs = [yrows(16 * f1 + f2) for f1 in range(8)]
    yin = []
    for (rr, ri, sg) in locs:
        yin.append(((f32(y_ref[pl.ds(qrow + rr, 8), :]), 1), (f32(y_ref[pl.ds(qrow + ri, 8), :]), sg)))
    A = dft(yin, 1)
    for k1 in range(8):
        t = cmulc(A[k1], *croot(f2 * k1, N, 1))
        rr, ri, _ = locs[k1]
        y_ref[pl.ds(qrow + rr, 8), :] = u32(vmat(t[0]))
        y_ref[pl.ds(qrow + ri, 8), :] = u32(vmat(t[1]))


def _ld(y_ref, r):
    return (f32(y_ref[pl.ds(r, 8), :]), 1)


def ifft_emit(s_ref, st_ref, srow, k1, k2, y, is_gate):
    n = k1 + 8 * k2
    if n < KT - 1:
        return
    m = n - (KT - 1)
    for part in range(2):
        v = jnp.tanh(vmat(y[part]))
        idx = pl.ds(srow + (2 * m + part), 8, stride=2 * L)
        if is_gate:
            v = s_ref[idx, :] * (0.5 * v + 0.5)
        s_ref[idx, :] = v


def ifft_passB(y_ref, s_ref, st_ref, srow, qrow, k1, is_gate):
    tin = []
    for f2 in range(16):
        rr, ri, _ = yrows(16 * k1 + f2)
        tin.append((_ld(y_ref, qrow + rr), _ld(y_ref, qrow + ri)))
    Y = dft(tin, 1)
    for k2 in range(16):
        ifft_emit(s_ref, st_ref, srow, k1, k2, Y[k2], is_gate)


def ifft_passB1(y_ref, qrow, k1):
    locs = [yrows(16 * k1 + f2) for f2 in range(1, 16, 2)]
    O = dft([(_ld(y_ref, qrow + rr), _ld(y_ref, qrow + ri)) for rr, ri, _ in locs], 1)
    for k in range(8):
        t = cmulc(O[k], *croot(k, 16, 1))
        rr, ri, _ = locs[k]
        y_ref[pl.ds(qrow + rr, 8), :] = u32(vmat(t[0]))
        y_ref[pl.ds(qrow + ri, 8), :] = u32(vmat(t[1]))


def ifft_passB2(y_ref, s_ref, st_ref, srow, qrow, k1, is_gate):
    le = [yrows(16 * k1 + f2) for f2 in range(0, 16, 2)]
    lo = [yrows(16 * k1 + f2) for f2 in range(1, 16, 2)]
    E = dft([(_ld(y_ref, qrow + rr), _ld(y_ref, qrow + ri)) for rr, ri, _ in le], 1)
    for k in range(8):
        rr, ri, _ = lo[k]
        o = (_ld(y_ref, qrow + rr), _ld(y_ref, qrow + ri))
        if k1 + 8 * k >= KT - 1:
            ifft_emit(s_ref, st_ref, srow, k1, k, cadd(E[k], o), is_gate)
        ifft_emit(s_ref, st_ref, srow, k1, k + 8, csub(E[k], o), is_gate)


def convert(s_ref, ob_ref, q):
    srow = pl.multiple_of(q * (16 * L), 16) if not isinstance(q, int) else q * 16 * L
    obv = ob_ref.at[pl.ds(srow, 16 * L)]
    for i in range(L):
        obv[pl.ds(16 * i, 16), :] = bf(s_ref[pl.ds(srow + 16 * i, 16), :])


def ifft_pieces(y_ref, s_ref, st_ref, ob_ref, q, is_gate, ga, gb, lagcv=False):
    qrow = pl.multiple_of(q * 16, 16)
    srow = pl.multiple_of(q * (16 * L), 16)
    pieces = []
    for f0 in range(0, 16, ga):
        def pa(f0=f0):
            for f2 in range(f0, f0 + ga):
                ifft_passA(y_ref, qrow, f2)
        pieces.append(pa)
    if gb == 0:
        for k1 in range(8):
            pieces.append(lambda k1=k1: ifft_passB1(y_ref, qrow, k1))
            pieces.append(lambda k1=k1: ifft_passB2(y_ref, s_ref, st_ref, srow, qrow, k1, is_gate))
        gb = 99
    for k0 in range(0, 8 if gb != 99 else 0, gb):
        def pb(k0=k0):
            for k1 in range(k0, k0 + gb):
                ifft_passB(y_ref, s_ref, st_ref, srow, qrow, k1, is_gate)
        pieces.append(pb)
    if is_gate and not lagcv:
        pieces.append(lambda: convert(s_ref, ob_ref, q))
    return pieces


LANE0 = (0, 256, 128, 384)
RT = 16 * L
VB = 2 * BSTR


T5 = (0, 40, 80, 120, 160)
CFG0 = {
    "": (1, 2, 1, 1, 1, T5),
    "W": (1, 2, 1, 1, 3, T5),
    "F": (0, 3, 1, 1, 1, T5),
    "G": (1, 2, 1, 1, 1, T5),
    "FW": (1, 2, 2, 2, 2, T5),
    "GW": (1, 2, 2, 2, 2, T5),
}


def make_kern(cfg=None, w0n=2, xp=4, xahead=2, tailb=(0, 5, 11, 15, 18, 20, 21), upto=99):
  CFG = dict(CFG0)
  if cfg:
    CFG.update(cfg)
  lagcv = True

  def kern(x_hbm, w_hbm, o_hbm, y0, y1, xh_ref, wh0, wh1, s_ref, st_ref, ws_ref, tw_ref, ob_ref, z_ref, xsem, wsem, osem, w0sem):
    ys = (y0, y1)
    whs = (wh0, wh1)
    xu = x_hbm.bitcast(jnp.uint32)
    wu = w_hbm.bitcast(jnp.uint32)

    XPIECE = 8000 // xp
    NXP = 2 * xp

    def xcp(p, h):
        b, i = divmod(p, xp)
        return pltpu.make_async_copy(xu.at[b, pl.ds(XPIECE * i, XPIECE), pl.ds(128 * h, 128)],
                                     ys[h].at[pl.ds(XOFF + b * BSTR + XPIECE * i, XPIECE)], xsem.at[2 * p + h])

    def wcp(c):
        return pltpu.make_async_copy(wu.at[:, :, pl.ds(LANE0[c], 128)], ws_ref.at[0], wsem.at[0])

    z_ref[0] = 0

    def w0cp(i):
        n = 128 // w0n
        return pltpu.make_async_copy(wu.at[:, pl.ds(n * i, n), pl.ds(LANE0[0], 128)], ws_ref.at[0, :, pl.ds(n * i, n), :], w0sem.at[i])
    for i in range(w0n):
        w0cp(i).start()
    XAHEAD = xahead
    for p in range(XAHEAD):
        for h in range(2):
            xcp(p, h).start()
    for h in range(2):
        ys[h][pl.ds(0, 32), :] = jnp.zeros((32, 128), jnp.uint32)
        ys[h][pl.ds(8032, 232), :] = jnp.zeros((232, 128), jnp.uint32)
        ys[h][pl.ds(16264, 232), :] = jnp.zeros((232, 128), jnp.uint32)

    def scale(c):
        return (0.5 if c % 2 == 1 else 1.0) / N

    def wt0_body(r, _):
        for i in range(w0n):
            @pl.when(r == i * (16 // w0n))
            def _():
                w0cp(i).wait()
        for p in wt_pieces(ws_ref.at[0], tw_ref, whs[0], r, scale(0)):
            p()
        return 0
    jax.lax.fori_loop(0, 16, wt0_body, 0)

    first_q = {}
    for p in range(NXP):
        b, i = divmod(p, xp)
        st = XOFF + b * BSTR + XPIECE * i
        first_q[p] = min(q for q in range(NQ) if 8 * L * q + 2 + 7 * L + N > st)

    def fwd_body(q, _):
        for p in range(NXP):
            @pl.when(q == first_q[p])
            def _():
                for h in range(2):
                    xcp(p, h).wait()
                if p + XAHEAD < NXP:
                    for h in range(2):
                        xcp(p + XAHEAD, h).start()
                if p == NXP - 1:
                    wcp(1).start()
        fwd_column(ys, xh_ref, q)
        return 0
    jax.lax.fori_loop(0, NQ, fwd_body, 0)

    xh_u = xh_ref.bitcast(jnp.uint32)

    def ocp(hh, b, t0, n, k):
        return pltpu.make_async_copy(ob_ref.at[pl.ds(VB * b + t0, n)], o_hbm.at[b, pl.ds(t0, n), pl.ds(128 * hh, 128)], osem.at[k])

    def paced(pieces, tokens, ref, zero_row, lead, on=True):
        n = len(pieces)
        if not on:
            tokens = []
        for k, p in enumerate(pieces):
            if tokens and k >= lead:
                tk = tokens[((k - lead) * len(tokens)) // (n - lead + 1)]
                ref[pl.ds(zero_row, 8), :] = tk if ref.dtype == jnp.float32 else u32(tk)
            p()

    def phase(c_mm, c_if, c_wt, ranges):
        is_gate = c_if is not None and c_if % 2 == 1
        if c_mm is not None:
            wh_u = whs[c_mm % 2].bitcast(jnp.uint32)
            mm_special(xh_u, wh_u, ys[c_mm % 2])
        if c_wt is not None:
            wcp(c_wt).wait()

        def body(q, with_wt):
            kind = ("" if c_if is None else "G" if is_gate else "F") + ("W" if with_wt else "")
            cgb, clead, cg1, cg2, cleadw, ctok = CFG[kind]
            tokens = []
            for s in range(3):
                tokens += mm_slot(xh_u, wh_u, ys[c_mm % 2], 3 * q + s, ctok)
            z = z_ref[0]
            if is_gate:
                convert(s_ref, ob_ref, jnp.maximum(q - 1, 0))
            if c_if is not None:
                yif = ys[c_if % 2]
                paced(ifft_pieces(yif, s_ref, st_ref, ob_ref, q, is_gate, 1, cgb, True), tokens, yif,
                      pl.multiple_of(YROWS + z, 8), clead)
            if with_wt:
                paced(wt_pieces(ws_ref.at[0], tw_ref, whs[c_wt % 2], q, scale(c_wt), cg1, cg2), tokens, tw_ref,
                      pl.multiple_of(TWROWS + z, 8), cleadw)

        for (q0, q1, after) in ranges:
            with_wt = c_wt is not None and q1 <= 16
            jax.lax.fori_loop(q0, q1, lambda q, _: (body(q, with_wt), 0)[1], 0)
            if after is not None:
                after()

    def nop():
        pass

    NA = 15 if lagcv else 16

    def out0_a():
        ocp(0, 0, 0, 16000, 0).start()
        ocp(0, 1, 0, NA * RT - VB, 1).start()

    def out0_b():
        if lagcv:
            convert(s_ref, ob_ref, NQ - 1)
        ocp(0, 1, NA * RT - VB, 16000 - (NA * RT - VB), 2).start()

    def out0_wait():
        ocp(0, 0, 0, 16000, 0).wait()
        ocp(0, 1, 0, NA * RT - VB, 1).wait()
        ocp(0, 1, NA * RT - VB, 16000 - (NA * RT - VB), 2).wait()

    def out1_pieces():
        pcs = []
        for k in range(len(tailb) - 1):
            lo, hi = tailb[k] * RT, tailb[k + 1] * RT
            cur = []
            for b in range(2):
                a, e = max(lo, VB * b), min(hi, VB * b + 16000)
                if e > a:
                    cur.append((b, a - VB * b, e - a))
            pcs.append(cur)
        return pcs

    def out1(k, wait):
        for n, pc in enumerate(out1_pieces()[k]):
            cp = ocp(1, *pc, 3 + 2 * k + n)
            if wait:
                cp.wait()
            else:
                cp.start()

    def fin():
        z = z_ref[0]
        r = pl.ds(pl.multiple_of(z * 16, 16), 16)
        r8 = pl.ds(pl.multiple_of(z * 8, 8), 8)
        acc = xh_ref[z, z, z, r, :].astype(jnp.float32) + whs[0][z, z, r, :].astype(jnp.float32) + whs[1][z, z, r, :].astype(jnp.float32)
        acc = acc + s_ref[r, :] + ob_ref[r, :].astype(jnp.float32)
        acc = acc + jnp.concatenate([f32(ys[0][r8, :]), f32(ys[1][r8, :])], axis=0) + tw_ref[r, :]
        ob_ref[pl.ds(0, 16), :] = bf(acc)
        o = pltpu.make_async_copy(ob_ref.at[pl.ds(0, 16)], o_hbm.at[0, pl.ds(0, 16), pl.ds(0, 128)], osem.at[7])
        o.start(); o.wait()
    if upto == 0:
        wcp(1).wait(); fin(); return
    phase(0, None, 1, [(0, 16, lambda: wcp(2).start()), (16, NQ, None)])
    if upto == 1:
        wcp(2).wait(); fin(); return
    phase(1, 0, 2, [(0, 16, lambda: wcp(3).start()), (16, NQ, None)])
    if upto == 2:
        wcp(3).wait(); fin(); return
    phase(2, 1, 3, [(0, 16, out0_a), (16, NQ, out0_b)])
    if upto == 3:
        out0_wait(); fin(); return
    phase(3, 2, None, [(0, NQ, None)])
    out0_wait()
    if upto == 4:
        fin(); return

    def tail_body(q, _):
        if lagcv:
            convert(s_ref, ob_ref, jnp.maximum(q - 1, 0))
        for p in ifft_pieces(ys[1], s_ref, st_ref, ob_ref, q, True, 16, 8, lagcv):
            p()
        return 0
    nseg = len(tailb) - 1

    def pick(i, vals):
        r = vals[-1]
        for k in range(len(vals) - 2, -1, -1):
            r = jnp.where(i == k, vals[k], r)
        return r

    def seg(i, _):
        if lagcv:
            lb = [0] + [min(b + 1, NQ) for b in tailb[1:]]
            jax.lax.fori_loop(pick(i, lb[:-1]), pick(i, lb[1:]), tail_body, 0)

            @pl.when(i == nseg - 1)
            def _():
                convert(s_ref, ob_ref, NQ - 1)
        else:
            jax.lax.fori_loop(pick(i, tailb[:-1]), pick(i, tailb[1:]), tail_body, 0)
        for k in range(nseg):
            @pl.when(i == k)
            def _():
                out1(k, False)
        return 0
    jax.lax.fori_loop(0, nseg, seg, 0)
    for k in range(nseg):
        out1(k, True)
  return kern


@jax.jit
def pallas_standalone__autoregressive_conv_wavernn__speech_kernel(x, w):
    kern = make_kern(**{"xp": 2, "xahead": 1})
    flags = None
    return pl.pallas_call(
        kern,
        in_specs=[pl.BlockSpec(memory_space=pl.ANY), pl.BlockSpec(memory_space=pl.ANY)],
        out_specs=pl.BlockSpec(memory_space=pl.ANY),
        out_shape=jax.ShapeDtypeStruct(x.shape, x.dtype),
        scratch_shapes=[
            pltpu.VMEM((YROWS + 8, 128), jnp.uint32), pltpu.VMEM((YROWS + 8, 128), jnp.uint32),
            pltpu.VMEM((NS, 3, 2, 336, 128), jnp.bfloat16),
            pltpu.VMEM((NS, 3, 256, 128), jnp.bfloat16),
            pltpu.VMEM((NS, 3, 256, 128), jnp.bfloat16),
            pltpu.VMEM((2 * VB, 128), jnp.float32),
            pltpu.VMEM((8, 128), jnp.float32),
            pltpu.VMEM((1, 31, 128, 128), jnp.uint32),
            pltpu.VMEM((TWROWS + 8, 128), jnp.float32),
            pltpu.VMEM((2 * VB, 128), jnp.bfloat16),
            pltpu.SMEM((1,), jnp.int32),
            pltpu.SemaphoreType.DMA((32,)), pltpu.SemaphoreType.DMA((2,)), pltpu.SemaphoreType.DMA((16,)), pltpu.SemaphoreType.DMA((8,)),
        ],
        compiler_params=pltpu.CompilerParams(vmem_limit_bytes=127 * 1024 * 1024, flags=flags),
    )(x, w)
```

```python
import math
import numpy as np
import jax
import jax.numpy as jnp
from jax.experimental import pallas as pl
from jax.experimental.pallas import tpu as pltpu

def vneg(a):
    return None if a is None else (a[0], -a[1])


def vadd(a, b):
    if a is None:
        return b
    if b is None:
        return a
    if a[1] > 0 and b[1] > 0:
        return (a[0] + b[0], 1)
    if a[1] > 0 and b[1] < 0:
        return (a[0] - b[0], 1)
    if a[1] < 0 and b[1] > 0:
        return (b[0] - a[0], 1)
    return (a[0] + b[0], -1)


def vsub(a, b):
    return vadd(a, vneg(b))


def vmulc(a, c):
    if a is None or c == 0.0:
        return None
    if c == 1.0:
        return a
    if c == -1.0:
        return vneg(a)
    return (a[0] * float(np.float32(c * a[1])), 1)


def vmat(a):
    return a[0] if a[1] > 0 else -a[0]


def cadd(a, b):
    return (vadd(a[0], b[0]), vadd(a[1], b[1]))


def csub(a, b):
    return (vsub(a[0], b[0]), vsub(a[1], b[1]))


def conj(a):
    return (a[0], vneg(a[1]))


def cmuli(a, s):
    return (vneg(a[1]), a[0]) if s > 0 else (a[1], vneg(a[0]))


def _snap(x):
    for v in (0.0, 1.0, -1.0):
        if abs(x - v) < 1e-12:
            return v
    return x


def croot(num, den, sgn):
    ang = sgn * 2.0 * math.pi * (num % den) / den
    return _snap(math.cos(ang)), _snap(math.sin(ang))


def cmulc(z, c, s):
    re, im = z
    if s == 0.0:
        return (vmulc(re, c), vmulc(im, c))
    if c == 0.0:
        return (vmulc(im, -s), vmulc(re, s))
    if im is None:
        return (vmulc(re, c), vmulc(re, s))
    if re is None:
        return (vmulc(im, -s), vmulc(im, c))
    if abs(abs(c) - abs(s)) < 1e-12:
        if s / c > 0:
            return (vmulc(vsub(re, im), c), vmulc(vadd(re, im), c))
        return (vmulc(vadd(re, im), c), vmulc(vsub(im, re), c))
    return (vsub(vmulc(re, c), vmulc(im, s)), vadd(vmulc(re, s), vmulc(im, c)))


def dft(xs, sgn):
    n = len(xs)
    if n == 1:
        return list(xs)
    if n == 2:
        return [cadd(xs[0], xs[1]), csub(xs[0], xs[1])]
    U = dft(xs[0::2], sgn)
    Z = dft(xs[1::4], sgn)
    Zp = dft(xs[3::4], sgn)
    out = [None] * n
    q = n // 4
    for k in range(q):
        t1 = cmulc(Z[k], *croot(k, n, sgn))
        t2 = cmulc(Zp[k], *croot(3 * k, n, sgn))
        s = cadd(t1, t2)
        d = cmuli(csub(t1, t2), sgn)
        out[k] = cadd(U[k], s)
        out[k + 2 * q] = csub(U[k], s)
        out[k + q] = cadd(U[k + q], d)
        out[k + 3 * q] = csub(U[k + q], d)
    return out


def rdft(xs):
    n = len(xs)
    if n == 1:
        return [(xs[0], None)]
    if n == 2:
        return [(vadd(xs[0], xs[1]), None), (vsub(xs[0], xs[1]), None)]
    E = rdft(xs[0::2])
    O = rdft(xs[1::2])
    out = [None] * (n // 2 + 1)
    for k in range(n // 4 + 1):
        t = cmulc(O[k], *croot(k, n, -1))
        out[k] = cadd(E[k], t)
        if k != n // 4:
            out[n // 2 - k] = conj(csub(E[k], t))
    return out


N = 128
KT = 31
L = N - KT + 1
NB = 84
NQ = 21
BSTR = NB * L
XOFF = 32
XROWS = 2 * BSTR + 32
TROWS = 8 * 8 * 2 * 16
XPIECE = 2000


def _slots():
    s = []
    for u in range(9):
        for k2 in range(8):
            if u == 0 and (k2 == 0 or k2 >= 4):
                continue
            if u == 8 and k2 > 3:
                continue
            s.append((u, k2))
    return s


SLOTS = _slots()
NG = len(SLOTS)
SP = NG
NS = NG + 1
SIDX = {uk: i for i, uk in enumerate(SLOTS)}
YROWS = NS * 672
TWROWS = 9 * 8 * 2 * 16


def f32(u):
    return pltpu.bitcast(u, jnp.float32)


def u32(v):
    return pltpu.bitcast(v, jnp.uint32)


def bf(v):
    return v.astype(jnp.bfloat16)


def fwd_pass1(xs_ref, q, n2):
    base = 2 + q * (8 * L)
    xin = []
    for n1 in range(16):
        u = xs_ref[pl.ds(base + 8 * n1 + n2, 8, stride=L), :]
        xin.append(((f32(u << 16), 1), (f32(u & jnp.uint32(0xFFFF0000)), 1)))
    X1 = dft(xin, -1)
    for u in range(8):
        top = cmulc(X1[u], *croot(n2 * u, N, -1))
        if u == 0:
            bt = cmulc(X1[8], *croot(n2 * 8, N, -1))
        else:
            c, s = croot(n2 * (16 - u) - 16 * n2, N, -1)
            bt = cmulc(conj(X1[16 - u]), c, -s)
        for ri in range(2):
            r0 = XROWS + ((u * 8 + n2) * 2 + ri) * 16
            xs_ref[pl.ds(r0, 8), :] = u32(vmat(top[ri]))
            xs_ref[pl.ds(r0 + 8, 8), :] = u32(vmat(bt[ri]))


def fwd_pass2(xs_ref, xh_ref, h, q, u):
    rows = pl.ds(pl.multiple_of(q * 16, 16), 16)
    zin = []
    for n2 in range(8):
        r0 = XROWS + ((u * 8 + n2) * 2) * 16
        zin.append(((f32(xs_ref[pl.ds(r0, 16), :]), 1), (f32(xs_ref[pl.ds(r0 + 16, 16), :]), 1)))
    X2 = dft(zin, -1)
    if u == 0:
        def half(k2, tb):
            return tuple((v[0][8 * tb:8 * tb + 8], v[1]) for v in X2[k2])

        def cat(p, q_):
            return bf(jnp.concatenate([vmat(p), vmat(q_)], axis=0))
        for t, k2 in enumerate((0, 4)):
            a, b = half(k2, 0)
            xh_ref[SP, t, h, rows, :] = cat(a, b)
        for (uu, k2, kp, tb) in [(0, k, 8 - k, 0) for k in (1, 2, 3)] + [(8, k, 7 - k, 1) for k in range(4)]:
            j = SIDX[uu, k2]
            a, b = half(k2, tb)
            a2, b2 = half(kp, tb)
            xh_ref[j, 0, h, rows, :] = cat(a, a2)
            xh_ref[j, 1, h, rows, :] = cat(b, vneg(b2))
            xh_ref[j, 2, h, rows, :] = cat(vadd(a, b), vsub(a2, b2))
        return
    for k2 in range(8):
        j = SIDX[u, k2]
        a, b = X2[k2]
        xh_ref[j, 0, h, rows, :] = bf(vmat(a))
        xh_ref[j, 1, h, rows, :] = bf(vmat(b))
        xh_ref[j, 2, h, rows, :] = bf(vmat(vadd(a, b)))


def fwd_column(xs, xh_ref, q):
    for n2 in range(8):
        for h in range(2):
            fwd_pass1(xs[h], q, n2)
    for u in range(8):
        for h in range(2):
            fwd_pass2(xs[h], xh_ref, h, q, u)


def _wt_nonzero():
    class _P:
        def __add__(self, o): return self
        __sub__ = __mul__ = __radd__ = __rsub__ = __rmul__ = __add__
    nz = {}
    for rr in range(8):
        Y = rdft([(_P(), 1) if rr + 8 * m < KT else None for m in range(16)])
        for u in range(9):
            t = cmulc(Y[u], *croot(rr * u, N, -1))
            for ri in range(2):
                nz[rr, u, ri] = t[ri] is not None
    return nz


WT_NONZERO = _wt_nonzero()


def wt_pieces(ws, tw_ref, wh_ref, r, scale, g1=2, g2=2):
    r8 = pl.ds(pl.multiple_of(r * 8, 8), 8)
    rows = pl.ds(pl.multiple_of(r * 16, 16), 16)

    def tap(j):
        if j >= KT:
            return None
        wv = pltpu.bitcast(ws[KT - 1 - j, r8, :], jnp.bfloat16)
        return (wv.astype(jnp.float32) * float(scale), 1)

    def p1(rr):
        Y = rdft([tap(rr + 8 * m) for m in range(16)])
        for u in range(9):
            t = cmulc(Y[u], *croot(rr * u, N, -1))
            for ri in range(2):
                if t[ri] is not None:
                    tw_ref[pl.ds(((u * 8 + rr) * 2 + ri) * 16, 16), :] = vmat(t[ri])

    def p2(u):
        def ld(rr, ri):
            if not WT_NONZERO[rr, u, ri]:
                return None
            return (tw_ref[pl.ds(((u * 8 + rr) * 2 + ri) * 16, 16), :], 1)
        if u == 0:
            X2 = rdft([ld(rr, 0) for rr in range(8)])
        else:
            X2 = dft([(ld(rr, 0), ld(rr, 1)) for rr in range(8)], -1)
        for k2 in range(8):
            if u == 0 and k2 in (0, 4):
                wh_ref[SP, k2 // 4, rows, :] = bf(vmat(X2[k2][0]))
            if (u, k2) not in SIDX:
                continue
            j = SIDX[u, k2]
            c, d = X2[k2]
            wh_ref[j, 0, rows, :] = bf(vmat(c))
            wh_ref[j, 1, rows, :] = bf(vmat(vsub(d, c)))
            wh_ref[j, 2, rows, :] = bf(vmat(vadd(c, d)))

    pieces = []
    for r0 in range(0, 8, g1):
        pieces.append(lambda r0=r0: [p1(rr) for rr in range(r0, r0 + g1)])
    us = [1, 2, 3, 4, 5, 6, 7, 0, 8]
    for i in range(0, 9, g2):
        pieces.append(lambda i=i: [p2(u) for u in us[i:i + g2]])
    return pieces


def _lhs(xh_u, j, t):
    return jnp.concatenate([pltpu.bitcast(xh_u[j, t, h], jnp.bfloat16) for h in range(2)], axis=1)


def _rhs(wh_u, j, t):
    return pltpu.bitcast(wh_u[j, t], jnp.bfloat16)


def _dot(a, b):
    return jnp.dot(a, b, preferred_element_type=jnp.float32)


def mm_slot(xh_u, wh_u, y_ref, j, token_rows):
    base = pl.multiple_of(j * 672, 16) if not isinstance(j, int) else j * 672
    rre, rim = pl.ds(base, 336), pl.ds(base + 336, 336)
    k1 = _dot(_lhs(xh_u, j, 2), _rhs(wh_u, j, 0))
    y_ref[rre, :] = u32(k1)
    k2 = _dot(_lhs(xh_u, j, 0), _rhs(wh_u, j, 1))
    y_ref[rim, :] = u32(f32(y_ref[rre, :]) + k2)
    k3 = _dot(_lhs(xh_u, j, 1), _rhs(wh_u, j, 2))
    y_ref[rre, :] = u32(f32(y_ref[rre, :]) - k3)
    return [k[r:r + 8] for k in (k1, k2, k3) for r in token_rows]


def mm_special(xh_u, wh_u, y_ref):
    for t in range(2):
        y_ref[pl.ds(SP * 672 + 336 * t, 336), :] = u32(_dot(_lhs(xh_u, SP, t), _rhs(wh_u, SP, t)))


def yrows(f):
    f2, f1 = f % 16, f // 16
    if f == 0:
        return SP * 672, SP * 672 + 8, 1
    if f == 64:
        return SP * 672 + 336, SP * 672 + 344, 1
    if 1 <= f2 <= 7:
        j, tb = SIDX[f2, f1], 0
    elif f2 >= 9:
        j, tb = SIDX[16 - f2, 7 - f1], 1
    elif f2 == 0:
        j, tb = (SIDX[0, f1], 0) if f1 < 4 else (SIDX[0, 8 - f1], 1)
    else:
        j, tb = (SIDX[8, f1], 0) if f1 <= 3 else (SIDX[8, 7 - f1], 1)
    r = j * 672 + 8 * tb
    return r, r + 336, (-1 if tb else 1)


def ifft_passA(y_ref, qrow, f2):
    locs = [yrows(16 * f1 + f2) for f1 in range(8)]
    yin = []
    for (rr, ri, sg) in locs:
        yin.append(((f32(y_ref[pl.ds(qrow + rr, 8), :]), 1), (f32(y_ref[pl.ds(qrow + ri, 8), :]), sg)))
    A = dft(yin, 1)
    for k1 in range(8):
        t = cmulc(A[k1], *croot(f2 * k1, N, 1))
        rr, ri, _ = locs[k1]
        y_ref[pl.ds(qrow + rr, 8), :] = u32(vmat(t[0]))
        y_ref[pl.ds(qrow + ri, 8), :] = u32(vmat(t[1]))


def _ld(y_ref, r):
    return (f32(y_ref[pl.ds(r, 8), :]), 1)


def ifft_emit(s_ref, srow, k1, k2, y, is_gate):
    n = k1 + 8 * k2
    if n < KT - 1:
        return
    m = n - (KT - 1)
    for part in range(2):
        v = jnp.tanh(vmat(y[part]))
        idx = pl.ds(srow + (2 * m + part), 8, stride=2 * L)
        if is_gate:
            v = s_ref[idx, :] * (0.5 * v + 0.5)
        s_ref[idx, :] = v


def ifft_passB(y_ref, s_ref, srow, qrow, k1, is_gate):
    tin = []
    for f2 in range(16):
        rr, ri, _ = yrows(16 * k1 + f2)
        tin.append((_ld(y_ref, qrow + rr), _ld(y_ref, qrow + ri)))
    Y = dft(tin, 1)
    for k2 in range(16):
        ifft_emit(s_ref, srow, k1, k2, Y[k2], is_gate)


def ifft_passB1(y_ref, qrow, k1):
    locs = [yrows(16 * k1 + f2) for f2 in range(1, 16, 2)]
    O = dft([(_ld(y_ref, qrow + rr), _ld(y_ref, qrow + ri)) for rr, ri, _ in locs], 1)
    for k in range(8):
        t = cmulc(O[k], *croot(k, 16, 1))
        rr, ri, _ = locs[k]
        y_ref[pl.ds(qrow + rr, 8), :] = u32(vmat(t[0]))
        y_ref[pl.ds(qrow + ri, 8), :] = u32(vmat(t[1]))


def ifft_passB2(y_ref, s_ref, srow, qrow, k1, is_gate):
    le = [yrows(16 * k1 + f2) for f2 in range(0, 16, 2)]
    lo = [yrows(16 * k1 + f2) for f2 in range(1, 16, 2)]
    E = dft([(_ld(y_ref, qrow + rr), _ld(y_ref, qrow + ri)) for rr, ri, _ in le], 1)
    for k in range(8):
        rr, ri, _ = lo[k]
        o = (_ld(y_ref, qrow + rr), _ld(y_ref, qrow + ri))
        if k1 + 8 * k >= KT - 1:
            ifft_emit(s_ref, srow, k1, k, cadd(E[k], o), is_gate)
        ifft_emit(s_ref, srow, k1, k + 8, csub(E[k], o), is_gate)


def convert(s_ref, ob_ref, q):
    srow = pl.multiple_of(q * (16 * L), 16) if not isinstance(q, int) else q * 16 * L
    obv = ob_ref.at[pl.ds(srow, 16 * L)]
    for i in range(L):
        obv[pl.ds(16 * i, 16), :] = bf(s_ref[pl.ds(srow + 16 * i, 16), :])


def ifft_pieces(y_ref, s_ref, q, is_gate, ga, gb):
    qrow = q * 16 if isinstance(q, int) else pl.multiple_of(q * 16, 16)
    srow = q * 16 * L if isinstance(q, int) else pl.multiple_of(q * (16 * L), 16)
    pieces = []
    for f0 in range(0, 16, ga):
        def pa(f0=f0):
            for f2 in range(f0, f0 + ga):
                ifft_passA(y_ref, qrow, f2)
        pieces.append(pa)
    if gb == 0:
        for k1 in range(8):
            pieces.append(lambda k1=k1: ifft_passB1(y_ref, qrow, k1))
            pieces.append(lambda k1=k1: ifft_passB2(y_ref, s_ref, srow, qrow, k1, is_gate))
        gb = 99
    for k0 in range(0, 8 if gb != 99 else 0, gb):
        def pb(k0=k0):
            for k1 in range(k0, k0 + gb):
                ifft_passB(y_ref, s_ref, srow, qrow, k1, is_gate)
        pieces.append(pb)
    return pieces


LANE0 = (0, 256, 128, 384)
RT = 16 * L
VB = 2 * BSTR


T5 = (0, 40, 80, 120, 160)
CFG0 = {
    "": (1, 2, 1, 1, 1, T5),
    "W": (1, 2, 1, 1, 3, T5),
    "F": (0, 3, 1, 1, 1, T5),
    "G": (1, 2, 1, 1, 1, T5),
    "FW": (1, 2, 2, 2, 2, T5),
    "GW": (1, 2, 2, 2, 2, T5),
}


def make_kern(cfg=None, unr=None, w0n=2, xp=2, xahead=1, tailb=(0, 4, 8, 11, 14, 17, 19, 20, 21)):
  CFG = dict(CFG0)
  if cfg:
    CFG.update(cfg)

  def kern(x_hbm, w_hbm, o_hbm, y0, y1, xh_ref, wh0, wh1, s_ref, ws_ref, tw_ref, ob_ref, z_ref, xsem, wsem, osem, w0sem):
    ys = (y0, y1)
    whs = (wh0, wh1)
    xu = x_hbm.bitcast(jnp.uint32)
    wu = w_hbm.bitcast(jnp.uint32)

    XPIECE = 8000 // xp
    NXP = 2 * xp

    def xcp(p, h):
        b, i = divmod(p, xp)
        return pltpu.make_async_copy(xu.at[b, pl.ds(XPIECE * i, XPIECE), pl.ds(128 * h, 128)],
                                     ys[h].at[pl.ds(XOFF + b * BSTR + XPIECE * i, XPIECE)], xsem.at[2 * p + h])

    def wcp(c):
        return pltpu.make_async_copy(wu.at[:, :, pl.ds(LANE0[c], 128)], ws_ref.at[0], wsem.at[0])

    z_ref[0] = 0

    def w0cp(i):
        n = 128 // w0n
        return pltpu.make_async_copy(wu.at[:, pl.ds(n * i, n), pl.ds(LANE0[0], 128)], ws_ref.at[0, :, pl.ds(n * i, n), :], w0sem.at[i])
    for i in range(w0n):
        w0cp(i).start()
    XAHEAD = xahead
    for p in range(XAHEAD):
        for h in range(2):
            xcp(p, h).start()
    for h in range(2):
        ys[h][pl.ds(0, 32), :] = jnp.zeros((32, 128), jnp.uint32)
        ys[h][pl.ds(8032, 232), :] = jnp.zeros((232, 128), jnp.uint32)
        ys[h][pl.ds(16264, 232), :] = jnp.zeros((232, 128), jnp.uint32)

    def scale(c):
        return (0.5 if c % 2 == 1 else 1.0) / N

    def wt0_body(r, _):
        for i in range(w0n):
            @pl.when(r == i * (16 // w0n))
            def _():
                w0cp(i).wait()
        for p in wt_pieces(ws_ref.at[0], tw_ref, whs[0], r, scale(0)):
            p()
        return 0
    jax.lax.fori_loop(0, 16, wt0_body, 0)

    first_q = {}
    for p in range(NXP):
        b, i = divmod(p, xp)
        st = XOFF + b * BSTR + XPIECE * i
        first_q[p] = min(q for q in range(NQ) if 8 * L * q + 2 + 7 * L + N > st)

    def fwd_body(q, _):
        for p in range(NXP):
            @pl.when(q == first_q[p])
            def _():
                for h in range(2):
                    xcp(p, h).wait()
                if p + XAHEAD < NXP:
                    for h in range(2):
                        xcp(p + XAHEAD, h).start()
                if p == NXP - 1:
                    wcp(1).start()
        fwd_column(ys, xh_ref, q)
        return 0
    jax.lax.fori_loop(0, NQ, fwd_body, 0)

    xh_u = xh_ref.bitcast(jnp.uint32)

    def ocp(hh, b, t0, n, k):
        return pltpu.make_async_copy(ob_ref.at[pl.ds(VB * b + t0, n)], o_hbm.at[b, pl.ds(t0, n), pl.ds(128 * hh, 128)], osem.at[k])

    def paced(pieces, tokens, ref, zero_row, lead, on=True):
        n = len(pieces)
        if not on:
            tokens = []
        for k, p in enumerate(pieces):
            if tokens and k >= lead:
                tk = tokens[((k - lead) * len(tokens)) // (n - lead + 1)]
                ref[pl.ds(zero_row, 8), :] = tk if ref.dtype == jnp.float32 else u32(tk)
            p()

    def phase(c_mm, c_if, c_wt, ranges):
        is_gate = c_if is not None and c_if % 2 == 1
        if c_mm is not None:
            wh_u = whs[c_mm % 2].bitcast(jnp.uint32)
            mm_special(xh_u, wh_u, ys[c_mm % 2])
        if c_wt is not None:
            wcp(c_wt).wait()

        def body(q, with_wt):
            kind = ("" if c_if is None else "G" if is_gate else "F") + ("W" if with_wt else "")
            cgb, clead, cg1, cg2, cleadw, ctok = CFG[kind]
            tokens = []
            for s in range(3):
                tokens += mm_slot(xh_u, wh_u, ys[c_mm % 2], 3 * q + s, ctok)
            z = z_ref[0]
            if is_gate:
                convert(s_ref, ob_ref, max(q - 1, 0) if isinstance(q, int) else jnp.maximum(q - 1, 0))
            if c_if is not None:
                yif = ys[c_if % 2]
                paced(ifft_pieces(yif, s_ref, q, is_gate, 1, cgb), tokens, yif,
                      pl.multiple_of(YROWS + z, 8), clead)
            if with_wt:
                paced(wt_pieces(ws_ref.at[0], tw_ref, whs[c_wt % 2], q, scale(c_wt), cg1, cg2), tokens, tw_ref,
                      pl.multiple_of(TWROWS + z, 8), cleadw)

        for (q0, q1, after) in ranges:
            with_wt = c_wt is not None and q1 <= 16
            kind = ("" if c_if is None else "G" if is_gate else "F") + ("W" if with_wt else "")
            u = (unr or {}).get(kind, 1)
            nfull = (q1 - q0) // u

            def bodyu(i, _):
                for t in range(u):
                    body(q0 + u * i + t, with_wt)
                return 0
            jax.lax.fori_loop(0, nfull, bodyu, 0)
            for qq in range(q0 + u * nfull, q1):
                body(qq, with_wt)
            if after is not None:
                after()

    NA = 15

    def out0_a():
        ocp(0, 0, 0, 16000, 0).start()
        ocp(0, 1, 0, NA * RT - VB, 1).start()

    def out0_b():
        convert(s_ref, ob_ref, NQ - 1)
        ocp(0, 1, NA * RT - VB, 16000 - (NA * RT - VB), 2).start()

    def out0_wait():
        ocp(0, 0, 0, 16000, 0).wait()
        ocp(0, 1, 0, NA * RT - VB, 1).wait()
        ocp(0, 1, NA * RT - VB, 16000 - (NA * RT - VB), 2).wait()

    def out1_pieces():
        pcs = []
        for k in range(len(tailb) - 1):
            lo, hi = tailb[k] * RT, tailb[k + 1] * RT
            cur = []
            for b in range(2):
                a, e = max(lo, VB * b), min(hi, VB * b + 16000)
                if e > a:
                    cur.append((b, a - VB * b, e - a))
            pcs.append(cur)
        return pcs

    def out1(k, wait):
        for n, pc in enumerate(out1_pieces()[k]):
            cp = ocp(1, *pc, 3 + 2 * k + n)
            if wait:
                cp.wait()
            else:
                cp.start()

    phase(0, None, 1, [(0, 16, lambda: wcp(2).start()), (16, NQ, None)])
    phase(1, 0, 2, [(0, 16, lambda: wcp(3).start()), (16, NQ, None)])
    phase(2, 1, 3, [(0, 16, out0_a), (16, NQ, out0_b)])
    phase(3, 2, None, [(0, NQ, None)])
    out0_wait()

    def tail_body(q, _):
        convert(s_ref, ob_ref, jnp.maximum(q - 1, 0))
        for p in ifft_pieces(ys[1], s_ref, q, True, 16, 8):
            p()
        return 0
    nseg = len(tailb) - 1

    def pick(i, vals):
        r = vals[-1]
        for k in range(len(vals) - 2, -1, -1):
            r = jnp.where(i == k, vals[k], r)
        return r

    def seg(i, _):
        lb = [0] + [min(b + 1, NQ) for b in tailb[1:]]
        jax.lax.fori_loop(pick(i, lb[:-1]), pick(i, lb[1:]), tail_body, 0)

        @pl.when(i == nseg - 1)
        def _():
            convert(s_ref, ob_ref, NQ - 1)
        for k in range(nseg):
            @pl.when(i == k)
            def _():
                out1(k, False)
        return 0
    jax.lax.fori_loop(0, nseg, seg, 0)
    for k in range(nseg):
        out1(k, True)
  return kern


@jax.jit
def pallas_standalone__autoregressive_conv_wavernn__speech_kernel(
    x: jax.Array,
    w: jax.Array,
):
    assert x.shape == (2, 16000, 256) and w.shape == (KT, 256, 512)
    kern = make_kern(unr={"F": 2, "G": 2, "": 2, "W": 2})
    return pl.pallas_call(
        kern,
        in_specs=[pl.BlockSpec(memory_space=pl.ANY), pl.BlockSpec(memory_space=pl.ANY)],
        out_specs=pl.BlockSpec(memory_space=pl.ANY),
        out_shape=jax.ShapeDtypeStruct(x.shape, x.dtype),
        scratch_shapes=[
            pltpu.VMEM((YROWS + 8, 128), jnp.uint32), pltpu.VMEM((YROWS + 8, 128), jnp.uint32),
            pltpu.VMEM((NS, 3, 2, 336, 128), jnp.bfloat16),
            pltpu.VMEM((NS, 3, 256, 128), jnp.bfloat16),
            pltpu.VMEM((NS, 3, 256, 128), jnp.bfloat16),
            pltpu.VMEM((2 * VB, 128), jnp.float32),
            pltpu.VMEM((1, 31, 128, 128), jnp.uint32),
            pltpu.VMEM((TWROWS + 8, 128), jnp.float32),
            pltpu.VMEM((2 * VB, 128), jnp.bfloat16),
            pltpu.SMEM((1,), jnp.int32),
            pltpu.SemaphoreType.DMA((8,)), pltpu.SemaphoreType.DMA((1,)), pltpu.SemaphoreType.DMA((20,)), pltpu.SemaphoreType.DMA((2,)),
        ],
        compiler_params=pltpu.CompilerParams(vmem_limit_bytes=127 * 1024 * 1024),
    )(x, w)
```

```python
import math
import numpy as np
import jax
import jax.numpy as jnp
from jax.experimental import pallas as pl
from jax.experimental.pallas import tpu as pltpu

def vneg(a):
    return None if a is None else (a[0], -a[1])


def vadd(a, b):
    if a is None:
        return b
    if b is None:
        return a
    if a[1] > 0 and b[1] > 0:
        return (a[0] + b[0], 1)
    if a[1] > 0 and b[1] < 0:
        return (a[0] - b[0], 1)
    if a[1] < 0 and b[1] > 0:
        return (b[0] - a[0], 1)
    return (a[0] + b[0], -1)


def vsub(a, b):
    return vadd(a, vneg(b))


def vmulc(a, c):
    if a is None or c == 0.0:
        return None
    if c == 1.0:
        return a
    if c == -1.0:
        return vneg(a)
    return (a[0] * float(np.float32(c * a[1])), 1)


def vmat(a):
    return a[0] if a[1] > 0 else -a[0]


def cadd(a, b):
    return (vadd(a[0], b[0]), vadd(a[1], b[1]))


def csub(a, b):
    return (vsub(a[0], b[0]), vsub(a[1], b[1]))


def conj(a):
    return (a[0], vneg(a[1]))


def cmuli(a, s):
    return (vneg(a[1]), a[0]) if s > 0 else (a[1], vneg(a[0]))


def _snap(x):
    for v in (0.0, 1.0, -1.0):
        if abs(x - v) < 1e-12:
            return v
    return x


def croot(num, den, sgn):
    ang = sgn * 2.0 * math.pi * (num % den) / den
    return _snap(math.cos(ang)), _snap(math.sin(ang))


def cmulc(z, c, s):
    re, im = z
    if s == 0.0:
        return (vmulc(re, c), vmulc(im, c))
    if c == 0.0:
        return (vmulc(im, -s), vmulc(re, s))
    if im is None:
        return (vmulc(re, c), vmulc(re, s))
    if re is None:
        return (vmulc(im, -s), vmulc(im, c))
    if abs(abs(c) - abs(s)) < 1e-12:
        if s / c > 0:
            return (vmulc(vsub(re, im), c), vmulc(vadd(re, im), c))
        return (vmulc(vadd(re, im), c), vmulc(vsub(im, re), c))
    return (vsub(vmulc(re, c), vmulc(im, s)), vadd(vmulc(re, s), vmulc(im, c)))


def dft(xs, sgn):
    n = len(xs)
    if n == 1:
        return list(xs)
    if n == 2:
        return [cadd(xs[0], xs[1]), csub(xs[0], xs[1])]
    U = dft(xs[0::2], sgn)
    Z = dft(xs[1::4], sgn)
    Zp = dft(xs[3::4], sgn)
    out = [None] * n
    q = n // 4
    for k in range(q):
        t1 = cmulc(Z[k], *croot(k, n, sgn))
        t2 = cmulc(Zp[k], *croot(3 * k, n, sgn))
        s = cadd(t1, t2)
        d = cmuli(csub(t1, t2), sgn)
        out[k] = cadd(U[k], s)
        out[k + 2 * q] = csub(U[k], s)
        out[k + q] = cadd(U[k + q], d)
        out[k + 3 * q] = csub(U[k + q], d)
    return out


def rdft(xs):
    n = len(xs)
    if n == 1:
        return [(xs[0], None)]
    if n == 2:
        return [(vadd(xs[0], xs[1]), None), (vsub(xs[0], xs[1]), None)]
    E = rdft(xs[0::2])
    O = rdft(xs[1::2])
    out = [None] * (n // 2 + 1)
    for k in range(n // 4 + 1):
        t = cmulc(O[k], *croot(k, n, -1))
        out[k] = cadd(E[k], t)
        if k != n // 4:
            out[n // 2 - k] = conj(csub(E[k], t))
    return out


N = 128
KT = 31
L = N - KT + 1
NB = 84
NQ = 21
BSTR = NB * L
XOFF = 32
XROWS = 2 * BSTR + 32
TROWS = 8 * 8 * 2 * 16
XPIECE = 2000


def _slots():
    s = []
    for u in range(9):
        for k2 in range(8):
            if u == 0 and (k2 == 0 or k2 >= 4):
                continue
            if u == 8 and k2 > 3:
                continue
            s.append((u, k2))
    return s


SLOTS = _slots()
NG = len(SLOTS)
SP = NG
NS = NG + 1
SIDX = {uk: i for i, uk in enumerate(SLOTS)}
YROWS = NS * 672
TWROWS = 9 * 8 * 2 * 16


def f32(u):
    return pltpu.bitcast(u, jnp.float32)


def u32(v):
    return pltpu.bitcast(v, jnp.uint32)


def bf(v):
    return v.astype(jnp.bfloat16)


def fwd_pass1(xs_ref, q, n2):
    base = 2 + q * (8 * L)
    xin = []
    for n1 in range(16):
        u = xs_ref[pl.ds(base + 8 * n1 + n2, 8, stride=L), :]
        xin.append(((f32(u << 16), 1), (f32(u & jnp.uint32(0xFFFF0000)), 1)))
    X1 = dft(xin, -1)
    for u in range(8):
        top = cmulc(X1[u], *croot(n2 * u, N, -1))
        if u == 0:
            bt = cmulc(X1[8], *croot(n2 * 8, N, -1))
        else:
            c, s = croot(n2 * (16 - u) - 16 * n2, N, -1)
            bt = cmulc(conj(X1[16 - u]), c, -s)
        for ri in range(2):
            r0 = XROWS + ((u * 8 + n2) * 2 + ri) * 16
            xs_ref[pl.ds(r0, 8), :] = u32(vmat(top[ri]))
            xs_ref[pl.ds(r0 + 8, 8), :] = u32(vmat(bt[ri]))


def fwd_pass2(xs_ref, xh_ref, h, q, u):
    rows = pl.ds(pl.multiple_of(q * 16, 16), 16)
    zin = []
    for n2 in range(8):
        r0 = XROWS + ((u * 8 + n2) * 2) * 16
        zin.append(((f32(xs_ref[pl.ds(r0, 16), :]), 1), (f32(xs_ref[pl.ds(r0 + 16, 16), :]), 1)))
    X2 = dft(zin, -1)
    if u == 0:
        def half(k2, tb):
            return tuple((v[0][8 * tb:8 * tb + 8], v[1]) for v in X2[k2])

        def cat(p, q_):
            return bf(jnp.concatenate([vmat(p), vmat(q_)], axis=0))
        for t, k2 in enumerate((0, 4)):
            a, b = half(k2, 0)
            xh_ref[SP, t, h, rows, :] = cat(a, b)
        for (uu, k2, kp, tb) in [(0, k, 8 - k, 0) for k in (1, 2, 3)] + [(8, k, 7 - k, 1) for k in range(4)]:
            j = SIDX[uu, k2]
            a, b = half(k2, tb)
            a2, b2 = half(kp, tb)
            xh_ref[j, 0, h, rows, :] = cat(a, a2)
            xh_ref[j, 1, h, rows, :] = cat(b, vneg(b2))
            xh_ref[j, 2, h, rows, :] = cat(vadd(a, b), vsub(a2, b2))
        return
    for k2 in range(8):
        j = SIDX[u, k2]
        a, b = X2[k2]
        xh_ref[j, 0, h, rows, :] = bf(vmat(a))
        xh_ref[j, 1, h, rows, :] = bf(vmat(b))
        xh_ref[j, 2, h, rows, :] = bf(vmat(vadd(a, b)))


def fwd_column(xs, xh_ref, q):
    for n2 in range(8):
        for h in range(2):
            fwd_pass1(xs[h], q, n2)
    for u in range(8):
        for h in range(2):
            fwd_pass2(xs[h], xh_ref, h, q, u)


def _wt_nonzero():
    class _P:
        def __add__(self, o): return self
        __sub__ = __mul__ = __radd__ = __rsub__ = __rmul__ = __add__
    nz = {}
    for rr in range(8):
        Y = rdft([(_P(), 1) if rr + 8 * m < KT else None for m in range(16)])
        for u in range(9):
            t = cmulc(Y[u], *croot(rr * u, N, -1))
            for ri in range(2):
                nz[rr, u, ri] = t[ri] is not None
    return nz


WT_NONZERO = _wt_nonzero()


def wt_pieces(ws, tw_ref, wh_ref, r, scale, g1=2, g2=2):
    r8 = pl.ds(pl.multiple_of(r * 8, 8), 8)
    rows = pl.ds(pl.multiple_of(r * 16, 16), 16)

    def tap(j):
        if j >= KT:
            return None
        wv = pltpu.bitcast(ws[KT - 1 - j, r8, :], jnp.bfloat16)
        return (wv.astype(jnp.float32) * float(scale), 1)

    def p1(rr):
        Y = rdft([tap(rr + 8 * m) for m in range(16)])
        for u in range(9):
            t = cmulc(Y[u], *croot(rr * u, N, -1))
            for ri in range(2):
                if t[ri] is not None:
                    tw_ref[pl.ds(((u * 8 + rr) * 2 + ri) * 16, 16), :] = vmat(t[ri])

    def p2(u):
        def ld(rr, ri):
            if not WT_NONZERO[rr, u, ri]:
                return None
            return (tw_ref[pl.ds(((u * 8 + rr) * 2 + ri) * 16, 16), :], 1)
        if u == 0:
            X2 = rdft([ld(rr, 0) for rr in range(8)])
        else:
            X2 = dft([(ld(rr, 0), ld(rr, 1)) for rr in range(8)], -1)
        for k2 in range(8):
            if u == 0 and k2 in (0, 4):
                wh_ref[SP, k2 // 4, rows, :] = bf(vmat(X2[k2][0]))
            if (u, k2) not in SIDX:
                continue
            j = SIDX[u, k2]
            c, d = X2[k2]
            wh_ref[j, 0, rows, :] = bf(vmat(c))
            wh_ref[j, 1, rows, :] = bf(vmat(vsub(d, c)))
            wh_ref[j, 2, rows, :] = bf(vmat(vadd(c, d)))

    pieces = []
    for r0 in range(0, 8, g1):
        pieces.append(lambda r0=r0: [p1(rr) for rr in range(r0, r0 + g1)])
    us = [1, 2, 3, 4, 5, 6, 7, 0, 8]
    for i in range(0, 9, g2):
        pieces.append(lambda i=i: [p2(u) for u in us[i:i + g2]])
    return pieces


def _lhs(xh_u, j, t):
    return jnp.concatenate([pltpu.bitcast(xh_u[j, t, h], jnp.bfloat16) for h in range(2)], axis=1)


def _rhs(wh_u, j, t):
    return pltpu.bitcast(wh_u[j, t], jnp.bfloat16)


def _dot(a, b):
    return jnp.dot(a, b, preferred_element_type=jnp.float32)


def mm_slot(xh_u, wh_u, y_ref, j, token_rows):
    base = pl.multiple_of(j * 672, 16) if not isinstance(j, int) else j * 672
    rre, rim = pl.ds(base, 336), pl.ds(base + 336, 336)
    k1 = _dot(_lhs(xh_u, j, 2), _rhs(wh_u, j, 0))
    y_ref[rre, :] = u32(k1)
    k2 = _dot(_lhs(xh_u, j, 0), _rhs(wh_u, j, 1))
    y_ref[rim, :] = u32(f32(y_ref[rre, :]) + k2)
    k3 = _dot(_lhs(xh_u, j, 1), _rhs(wh_u, j, 2))
    y_ref[rre, :] = u32(f32(y_ref[rre, :]) - k3)
    return [k[r:r + 8] for k in (k1, k2, k3) for r in token_rows]


def mm_special(xh_u, wh_u, y_ref):
    for t in range(2):
        y_ref[pl.ds(SP * 672 + 336 * t, 336), :] = u32(_dot(_lhs(xh_u, SP, t), _rhs(wh_u, SP, t)))


def yrows(f):
    f2, f1 = f % 16, f // 16
    if f == 0:
        return SP * 672, SP * 672 + 8, 1
    if f == 64:
        return SP * 672 + 336, SP * 672 + 344, 1
    if 1 <= f2 <= 7:
        j, tb = SIDX[f2, f1], 0
    elif f2 >= 9:
        j, tb = SIDX[16 - f2, 7 - f1], 1
    elif f2 == 0:
        j, tb = (SIDX[0, f1], 0) if f1 < 4 else (SIDX[0, 8 - f1], 1)
    else:
        j, tb = (SIDX[8, f1], 0) if f1 <= 3 else (SIDX[8, 7 - f1], 1)
    r = j * 672 + 8 * tb
    return r, r + 336, (-1 if tb else 1)


def ifft_passA(y_ref, qrow, f2):
    locs = [yrows(16 * f1 + f2) for f1 in range(8)]
    yin = []
    for (rr, ri, sg) in locs:
        yin.append(((f32(y_ref[pl.ds(qrow + rr, 8), :]), 1), (f32(y_ref[pl.ds(qrow + ri, 8), :]), sg)))
    A = dft(yin, 1)
    for k1 in range(8):
        t = cmulc(A[k1], *croot(f2 * k1, N, 1))
        rr, ri, _ = locs[k1]
        y_ref[pl.ds(qrow + rr, 8), :] = u32(vmat(t[0]))
        y_ref[pl.ds(qrow + ri, 8), :] = u32(vmat(t[1]))


def _ld(y_ref, r):
    return (f32(y_ref[pl.ds(r, 8), :]), 1)


def ifft_emit(s_ref, srow, k1, k2, y, is_gate):
    n = k1 + 8 * k2
    if n < KT - 1:
        return
    m = n - (KT - 1)
    for part in range(2):
        v = jnp.tanh(vmat(y[part]))
        idx = pl.ds(srow + (2 * m + part), 8, stride=2 * L)
        if is_gate:
            v = s_ref[idx, :] * (0.5 * v + 0.5)
        s_ref[idx, :] = v


def ifft_passB(y_ref, s_ref, srow, qrow, k1, is_gate):
    tin = []
    for f2 in range(16):
        rr, ri, _ = yrows(16 * k1 + f2)
        tin.append((_ld(y_ref, qrow + rr), _ld(y_ref, qrow + ri)))
    Y = dft(tin, 1)
    for k2 in range(16):
        ifft_emit(s_ref, srow, k1, k2, Y[k2], is_gate)


def ifft_passB1(y_ref, qrow, k1):
    locs = [yrows(16 * k1 + f2) for f2 in range(1, 16, 2)]
    O = dft([(_ld(y_ref, qrow + rr), _ld(y_ref, qrow + ri)) for rr, ri, _ in locs], 1)
    for k in range(8):
        t = cmulc(O[k], *croot(k, 16, 1))
        rr, ri, _ = locs[k]
        y_ref[pl.ds(qrow + rr, 8), :] = u32(vmat(t[0]))
        y_ref[pl.ds(qrow + ri, 8), :] = u32(vmat(t[1]))


def ifft_passB2(y_ref, s_ref, srow, qrow, k1, is_gate):
    le = [yrows(16 * k1 + f2) for f2 in range(0, 16, 2)]
    lo = [yrows(16 * k1 + f2) for f2 in range(1, 16, 2)]
    E = dft([(_ld(y_ref, qrow + rr), _ld(y_ref, qrow + ri)) for rr, ri, _ in le], 1)
    for k in range(8):
        rr, ri, _ = lo[k]
        o = (_ld(y_ref, qrow + rr), _ld(y_ref, qrow + ri))
        if k1 + 8 * k >= KT - 1:
            ifft_emit(s_ref, srow, k1, k, cadd(E[k], o), is_gate)
        ifft_emit(s_ref, srow, k1, k + 8, csub(E[k], o), is_gate)


def convert(s_ref, ob_ref, q):
    srow = pl.multiple_of(q * (16 * L), 16) if not isinstance(q, int) else q * 16 * L
    obv = ob_ref.at[pl.ds(srow, 16 * L)]
    for i in range(L):
        obv[pl.ds(16 * i, 16), :] = bf(s_ref[pl.ds(srow + 16 * i, 16), :])


def ifft_pieces(y_ref, s_ref, q, is_gate, ga, gb):
    qrow = q * 16 if isinstance(q, int) else pl.multiple_of(q * 16, 16)
    srow = q * 16 * L if isinstance(q, int) else pl.multiple_of(q * (16 * L), 16)
    pieces = []
    for f0 in range(0, 16, ga):
        def pa(f0=f0):
            for f2 in range(f0, f0 + ga):
                ifft_passA(y_ref, qrow, f2)
        pieces.append(pa)
    if gb == 0:
        for k1 in range(8):
            pieces.append(lambda k1=k1: ifft_passB1(y_ref, qrow, k1))
            pieces.append(lambda k1=k1: ifft_passB2(y_ref, s_ref, srow, qrow, k1, is_gate))
        gb = 99
    for k0 in range(0, 8 if gb != 99 else 0, gb):
        def pb(k0=k0):
            for k1 in range(k0, k0 + gb):
                ifft_passB(y_ref, s_ref, srow, qrow, k1, is_gate)
        pieces.append(pb)
    return pieces


LANE0 = (0, 256, 128, 384)
RT = 16 * L
VB = 2 * BSTR


T4 = (0, 48, 96, 160)
T5 = (0, 40, 80, 120, 160)
CFG0 = {
    "": (1, 2, 1, 1, 1, T5),
    "W": (1, 2, 1, 1, 3, T4),
    "F": (0, 3, 1, 1, 1, T4),
    "G": (0, 3, 1, 1, 1, T4),
    "FW": (0, 3, 2, 2, 2, T4),
    "GW": (1, 2, 2, 2, 2, T5),
}


def make_kern(cfg=None, unr=None, w0n=2, xp=2, xahead=1, tailb=(0, 4, 8, 11, 14, 17, 19, 20, 21)):
  CFG = dict(CFG0)
  if cfg:
    CFG.update(cfg)

  def kern(x_hbm, w_hbm, o_hbm, y0, y1, xh_ref, wh0, wh1, s_ref, ws_ref, tw_ref, ob_ref, z_ref, xsem, wsem, osem, w0sem):
    ys = (y0, y1)
    whs = (wh0, wh1)
    xu = x_hbm.bitcast(jnp.uint32)
    wu = w_hbm.bitcast(jnp.uint32)

    XPIECE = 8000 // xp
    NXP = 2 * xp

    def xcp(p, h):
        b, i = divmod(p, xp)
        return pltpu.make_async_copy(xu.at[b, pl.ds(XPIECE * i, XPIECE), pl.ds(128 * h, 128)],
                                     ys[h].at[pl.ds(XOFF + b * BSTR + XPIECE * i, XPIECE)], xsem.at[2 * p + h])

    def wcp(c):
        return pltpu.make_async_copy(wu.at[:, :, pl.ds(LANE0[c], 128)], ws_ref.at[0], wsem.at[0])

    z_ref[0] = 0

    def w0cp(i):
        n = 128 // w0n
        return pltpu.make_async_copy(wu.at[:, pl.ds(n * i, n), pl.ds(LANE0[0], 128)], ws_ref.at[0, :, pl.ds(n * i, n), :], w0sem.at[i])
    for i in range(w0n):
        w0cp(i).start()
    XAHEAD = xahead
    for p in range(XAHEAD):
        for h in range(2):
            xcp(p, h).start()
    for h in range(2):
        ys[h][pl.ds(0, 32), :] = jnp.zeros((32, 128), jnp.uint32)
        ys[h][pl.ds(8032, 232), :] = jnp.zeros((232, 128), jnp.uint32)
        ys[h][pl.ds(16264, 232), :] = jnp.zeros((232, 128), jnp.uint32)

    def scale(c):
        return (0.5 if c % 2 == 1 else 1.0) / N

    def wt0_body(r, _):
        for i in range(w0n):
            @pl.when(r == i * (16 // w0n))
            def _():
                w0cp(i).wait()
        for p in wt_pieces(ws_ref.at[0], tw_ref, whs[0], r, scale(0)):
            p()
        return 0
    jax.lax.fori_loop(0, 16, wt0_body, 0)

    first_q = {}
    for p in range(NXP):
        b, i = divmod(p, xp)
        st = XOFF + b * BSTR + XPIECE * i
        first_q[p] = min(q for q in range(NQ) if 8 * L * q + 2 + 7 * L + N > st)

    def fwd_body(q, _):
        for p in range(NXP):
            @pl.when(q == first_q[p])
            def _():
                for h in range(2):
                    xcp(p, h).wait()
                if p + XAHEAD < NXP:
                    for h in range(2):
                        xcp(p + XAHEAD, h).start()
                if p == NXP - 1:
                    wcp(1).start()
        fwd_column(ys, xh_ref, q)
        return 0
    jax.lax.fori_loop(0, NQ, fwd_body, 0)

    xh_u = xh_ref.bitcast(jnp.uint32)

    def ocp(hh, b, t0, n, k):
        return pltpu.make_async_copy(ob_ref.at[pl.ds(VB * b + t0, n)], o_hbm.at[b, pl.ds(t0, n), pl.ds(128 * hh, 128)], osem.at[k])

    def paced(pieces, tokens, ref, zero_row, lead, on=True):
        n = len(pieces)
        if not on:
            tokens = []
        for k, p in enumerate(pieces):
            if tokens and k >= lead:
                tk = tokens[((k - lead) * len(tokens)) // (n - lead + 1)]
                ref[pl.ds(zero_row, 8), :] = tk if ref.dtype == jnp.float32 else u32(tk)
            p()

    def phase(c_mm, c_if, c_wt, ranges):
        is_gate = c_if is not None and c_if % 2 == 1
        if c_mm is not None:
            wh_u = whs[c_mm % 2].bitcast(jnp.uint32)
            mm_special(xh_u, wh_u, ys[c_mm % 2])
        if c_wt is not None:
            wcp(c_wt).wait()

        def body(q, with_wt):
            kind = ("" if c_if is None else "G" if is_gate else "F") + ("W" if with_wt else "")
            cgb, clead, cg1, cg2, cleadw, ctok = CFG[kind]
            tokens = []
            for s in range(3):
                tokens += mm_slot(xh_u, wh_u, ys[c_mm % 2], 3 * q + s, ctok)
            z = z_ref[0]
            if is_gate:
                convert(s_ref, ob_ref, max(q - 1, 0) if isinstance(q, int) else jnp.maximum(q - 1, 0))
            if c_if is not None:
                yif = ys[c_if % 2]
                paced(ifft_pieces(yif, s_ref, q, is_gate, 1, cgb), tokens, yif,
                      pl.multiple_of(YROWS + z, 8), clead)
            if with_wt:
                paced(wt_pieces(ws_ref.at[0], tw_ref, whs[c_wt % 2], q, scale(c_wt), cg1, cg2), tokens, tw_ref,
                      pl.multiple_of(TWROWS + z, 8), cleadw)

        for (q0, q1, after) in ranges:
            with_wt = c_wt is not None and q1 <= 16
            kind = ("" if c_if is None else "G" if is_gate else "F") + ("W" if with_wt else "")
            u = (unr or {}).get(kind, 1)
            nfull = (q1 - q0) // u

            def bodyu(i, _):
                for t in range(u):
                    body(q0 + u * i + t, with_wt)
                return 0
            jax.lax.fori_loop(0, nfull, bodyu, 0)
            for qq in range(q0 + u * nfull, q1):
                body(qq, with_wt)
            if after is not None:
                after()

    NA = 15

    def out0_a():
        ocp(0, 0, 0, 16000, 0).start()
        ocp(0, 1, 0, NA * RT - VB, 1).start()

    def out0_b():
        convert(s_ref, ob_ref, NQ - 1)
        ocp(0, 1, NA * RT - VB, 16000 - (NA * RT - VB), 2).start()

    def out0_wait():
        ocp(0, 0, 0, 16000, 0).wait()
        ocp(0, 1, 0, NA * RT - VB, 1).wait()
        ocp(0, 1, NA * RT - VB, 16000 - (NA * RT - VB), 2).wait()

    def out1_pieces():
        pcs = []
        for k in range(len(tailb) - 1):
            lo, hi = tailb[k] * RT, tailb[k + 1] * RT
            cur = []
            for b in range(2):
                a, e = max(lo, VB * b), min(hi, VB * b + 16000)
                if e > a:
                    cur.append((b, a - VB * b, e - a))
            pcs.append(cur)
        return pcs

    def out1(k, wait):
        for n, pc in enumerate(out1_pieces()[k]):
            cp = ocp(1, *pc, 3 + 2 * k + n)
            if wait:
                cp.wait()
            else:
                cp.start()

    phase(0, None, 1, [(0, 16, lambda: wcp(2).start()), (16, NQ, None)])
    phase(1, 0, 2, [(0, 16, lambda: wcp(3).start()), (16, NQ, None)])
    phase(2, 1, 3, [(0, 16, out0_a), (16, NQ, out0_b)])
    phase(3, 2, None, [(0, NQ, None)])
    out0_wait()

    def tail_body(q, _):
        convert(s_ref, ob_ref, jnp.maximum(q - 1, 0))
        for p in ifft_pieces(ys[1], s_ref, q, True, 16, 8):
            p()
        return 0
    nseg = len(tailb) - 1

    def pick(i, vals):
        r = vals[-1]
        for k in range(len(vals) - 2, -1, -1):
            r = jnp.where(i == k, vals[k], r)
        return r

    def seg(i, _):
        lb = [0] + [min(b + 1, NQ) for b in tailb[1:]]
        jax.lax.fori_loop(pick(i, lb[:-1]), pick(i, lb[1:]), tail_body, 0)

        @pl.when(i == nseg - 1)
        def _():
            convert(s_ref, ob_ref, NQ - 1)
        for k in range(nseg):
            @pl.when(i == k)
            def _():
                out1(k, False)
        return 0
    jax.lax.fori_loop(0, nseg, seg, 0)
    for k in range(nseg):
        out1(k, True)
  return kern


@jax.jit
def pallas_standalone__autoregressive_conv_wavernn__speech_kernel(
    x: jax.Array,
    w: jax.Array,
):
    assert x.shape == (2, 16000, 256) and w.shape == (KT, 256, 512)
    kern = make_kern(unr={"F": 2, "G": 2, "": 2, "W": 2})
    return pl.pallas_call(
        kern,
        in_specs=[pl.BlockSpec(memory_space=pl.ANY), pl.BlockSpec(memory_space=pl.ANY)],
        out_specs=pl.BlockSpec(memory_space=pl.ANY),
        out_shape=jax.ShapeDtypeStruct(x.shape, x.dtype),
        scratch_shapes=[
            pltpu.VMEM((YROWS + 8, 128), jnp.uint32), pltpu.VMEM((YROWS + 8, 128), jnp.uint32),
            pltpu.VMEM((NS, 3, 2, 336, 128), jnp.bfloat16),
            pltpu.VMEM((NS, 3, 256, 128), jnp.bfloat16),
            pltpu.VMEM((NS, 3, 256, 128), jnp.bfloat16),
            pltpu.VMEM((2 * VB, 128), jnp.float32),
            pltpu.VMEM((1, 31, 128, 128), jnp.uint32),
            pltpu.VMEM((TWROWS + 8, 128), jnp.float32),
            pltpu.VMEM((2 * VB, 128), jnp.bfloat16),
            pltpu.SMEM((1,), jnp.int32),
            pltpu.SemaphoreType.DMA((8,)), pltpu.SemaphoreType.DMA((1,)), pltpu.SemaphoreType.DMA((20,)), pltpu.SemaphoreType.DMA((2,)),
        ],
        compiler_params=pltpu.CompilerParams(vmem_limit_bytes=127 * 1024 * 1024),
    )(x, w)
```
